```python
import os as _os
_os.environ.setdefault("JAX_PLATFORMS", "cpu")
import jax
import jax.numpy as jnp

def _softmax(x, axis=-1):
    return jax.nn.softmax(x, axis=axis)
def _gelu(x):
    return jax.nn.gelu(x, approximate=True)
def _silu(x):
    return jax.nn.silu(x)
def _sigmoid(x):
    return jax.nn.sigmoid(x)
def _layernorm(x, axis=-1, eps=1e-5):
    m = jnp.mean(x, axis=axis, keepdims=True)
    v = jnp.var(x, axis=axis, keepdims=True)
    return (x - m) / jnp.sqrt(v + eps)
def _scatter_add(tgt, idx, src, axis=0):
    return tgt.at[idx].add(src)
def _segment_sum(src, seg, n):
    return jax.ops.segment_sum(src, seg, n)
class _Rng:
    def __init__(self, key):
        self._k = key
    def _next(self):
        self._k, sub = jax.random.split(self._k)
        return sub
    def normal(self, shape):
        return jax.random.normal(self._next(), shape, dtype=jnp.bfloat16)
    def randint(self, lo, hi, shape):
        return jax.random.randint(self._next(), shape, lo, hi, dtype=jnp.int32)
    def uniform(self, shape, lo=0.0, hi=1.0):
        return jax.random.uniform(self._next(), shape, jnp.bfloat16, lo, hi)
    def permutation(self, n):
        return jax.random.permutation(self._next(), n)


kernel_name = 'concat_heads__linear_attn_block__ssm_conv_s4__prompt'

def setup_inputs():
    _rng = _Rng(jax.random.key(int.from_bytes(__import__("os").urandom(4), "little")))
    _w = (lambda a: (lambda t: t.astype(jnp.bfloat16) if jnp.issubdtype(t.dtype, jnp.floating) else t)(jnp.asarray(a)))
    def _A_setup():
        B, S, D = 1, 2048, 512
        return {
            "x": _w((lambda *s: _rng.normal(s) * 0.05)(B, S, D)),
            "wqkv": _w((lambda *s: _rng.normal(s) * 0.8)(D, 3 * D)),
            "wo": _w((lambda *s: _rng.normal(s) * 0.05)(D, D)),
        }
    _A_in = _A_setup()

    def _B_setup():
        B, L, D, N = 1, 2048, 512, 128
        A_re = -jnp.exp((lambda *s: _rng.normal(s) * 0.2)(D, N))
        A_im = jnp.pi * (lambda *s: _rng.normal(s) * 0.2)(D, N)
        B_re = (lambda *s: _rng.normal(s) * 0.2)(D, N)
        B_im = (lambda *s: _rng.normal(s) * 0.2)(D, N)
        C_re = (lambda *s: _rng.normal(s) * 0.2)(D, N)
        C_im = (lambda *s: _rng.normal(s) * 0.2)(D, N)
        log_dt = (lambda *s: _rng.normal(s) * 0.2)(D) * 0.5 - 4.0
        Dskip = (lambda *s: _rng.normal(s) * 0.05)(D)
        return {
            "u": _w((lambda *s: _rng.normal(s) * 0.05)(B, L, D)),
            "A_re": _w(A_re),
            "A_im": _w(A_im),
            "B_re": _w(B_re),
            "B_im": _w(B_im),
            "C_re": _w(C_re),
            "C_im": _w(C_im),
            "log_dt": _w(log_dt),
            "Dskip": _w(Dskip),
        }
    _B_in = _B_setup()

    return {
        "A_x": _A_in["x"],
        "A_wqkv": _A_in["wqkv"],
        "A_wo": _A_in["wo"],
        "B_u": _B_in["u"],
        "B_A_re": _B_in["A_re"],
        "B_A_im": _B_in["A_im"],
        "B_B_re": _B_in["B_re"],
        "B_B_im": _B_in["B_im"],
        "B_C_re": _B_in["C_re"],
        "B_C_im": _B_in["C_im"],
        "B_log_dt": _B_in["log_dt"],
        "B_Dskip": _B_in["Dskip"],
    }

def reference(A_x, A_wqkv, A_wo, B_u, B_A_re, B_A_im, B_B_re, B_B_im, B_C_re, B_C_im, B_log_dt, B_Dskip):
    def _A_ref(x, wqkv, wo):
        B, S, D = x.shape
        H = 32; Dh = D // H
        qkv = (lambda x, *d: x.transpose(*d))((x @ wqkv).reshape(B, S, 3, H, Dh), 2, 0, 3, 1, 4)
        q, k, v = qkv[0], qkv[1], qkv[2]
        phi = lambda t: jnp.where(t > 0, t + 1, jnp.exp(t)) + 1e-6
        pq, pk = phi(q), phi(k)
        kv = jnp.einsum("bhsd,bhse->bhde", pk, v)
        z = jnp.einsum("bhsd->bhd", pk)
        num = jnp.einsum("bhqd,bhde->bhqe", pq, kv)
        den = jnp.einsum("bhqd,bhd->bhq", pq, z)[..., None] + 1e-6
        o = num / den
        return (lambda x, *d: x.transpose(*d))(o, 0, 2, 1, 3).reshape(B, S, D) @ wo

    def _B_ref(u, A_re, A_im, B_re, B_im, C_re, C_im, log_dt, Dskip):
        Bsz, L, D = u.shape
        dt = jnp.exp(log_dt)[:, None]
        A = A_re + 1j * A_im
        Bc = B_re + 1j * B_im
        Cc = C_re + 1j * C_im
        logdA = dt * A
        dB = dt * Bc
        l = (lambda x, dt: x.astype(dt))(jnp.arange(L), A_re.dtype)
        P = jnp.exp(logdA[:, :, None] * l[None, None, :])
        K = jnp.einsum("dn,dnl,dn->dl", Cc, P, dB).real
        L2 = 2 * L
        Kp = jnp.pad(K, ((0, 0), (0, L)))
        up = (lambda x, *d: x.transpose(*d))(u, 0, 2, 1)
        up = jnp.pad(up, ((0, 0), (0, 0), (0, L)))
        Kf = (lambda x, axes=(-2,-1): jnp.fft.rfft2(x.astype(jnp.float32), axes=axes))(Kp[:, None, :], axes=(-2, -1))
        Uf = (lambda x, axes=(-2,-1): jnp.fft.rfft2(x.astype(jnp.float32), axes=axes))(up[:, :, None, :], axes=(-2, -1))
        Yf = Uf * Kf[None, :, :, :]
        y = (lambda x, s, axes=(-2,-1): jnp.fft.irfft2(x, s=s, axes=axes).astype(jnp.bfloat16))(Yf, (1, L2), axes=(-2, -1))[:, :, 0, :L]
        y = (lambda x, *d: x.transpose(*d))(y, 0, 2, 1) + u * Dskip[None, None, :]
        return y

    a = _A_ref(A_x, A_wqkv, A_wo)
    b = _B_ref(B_u, B_A_re, B_A_im, B_B_re, B_B_im, B_C_re, B_C_im, B_log_dt, B_Dskip)
    return jnp.concatenate([a, b], axis=-1)
```

```python
import functools

import jax
import jax.numpy as jnp
import numpy as np
from jax import lax
import jax.experimental.pallas as pl
import jax.experimental.pallas.tpu as pltpu

F32 = jnp.float32
BF16 = jnp.bfloat16
U32 = jnp.uint32

S = 2048
D = 512
T = 512


def _bf16_bits(x):
    u = np.ascontiguousarray(x, dtype=np.float32).view(np.uint32).astype(np.uint64)
    return (((u + 0x7FFF + ((u >> 16) & 1)) >> 16) & 0xFFFF).astype(np.uint32)


def _bf16_round_int(l):
    return int((_bf16_bits(np.array([l], np.float32)) << 16).view(np.float32)[0])


def _pack_rows(m):
    b = _bf16_bits(m)
    return (b[..., 0::2, :] | (b[..., 1::2, :] << 16)).astype(np.uint32)


_F_OF_ROW = np.array([2 * (8 * ((r // 8) % 8) + r % 8) + (r // 64) for r in range(128)])
_THETA = 2 * np.pi * (_F_OF_ROW + 0.5) / (2 * T)


def _fwd_col(m):
    c = np.cos(_THETA * m).reshape(16, 8)
    s = -np.sin(_THETA * m).reshape(16, 8)
    return np.concatenate([c, s], axis=1).reshape(256)


def _out_row_time(p, r):
    t2, s = r // 8, r % 8
    if (s % 2 == 0) == (p < 2):
        w, v = s, 0
    else:
        w, v = (s - 1) % 8, 1
    return 32 * t2 + 16 * v + 2 * w + (p % 2)


A_PAIRS = ((4, 2), (8, 6), (260, 258), (264, 262),
           (1, 516), (5, 520), (1544, 772), (1800, 776),
           (3, 1032), (7, 1288))
G_LIST = ((0, 0, 'TA0'), (0, 1, 'TA1'), (0, 2, 'TA2'), (0, 3, 'TA3'),
          (1, 0, 'TB'), (1, 3, 'TB'), (1, 1, 'TB1'), (1, 2, 'TB2'),
          (2, 0, 'TC'), (2, 2, 'TC'), (3, 0, 'TD'), (3, 2, 'TD'))
LANE_512, LANE_1024 = 6, 7


def _build_tiles(x1, y1, x2, y2, x3, y3, lane, where, roll):
    low_x = (lane % 8) < 4
    low_y = ((lane + 7) % 8) < 4
    return dict(
        TA0=x1,
        TA1=where(lane == LANE_512, roll(x1, 4), where(low_x, x2, x1)),
        TA2=y1,
        TA3=where(low_x, x3, x1),
        TB=y2,
        TB1=where(lane == LANE_1024, roll(x1, 1), y2),
        TB2=where(lane == LANE_512, x1, y2),
        TC=where(low_y, y3, y2),
        TD=where(low_x, y3, x2),
    )


@functools.lru_cache(maxsize=None)
def _tables():
    fu = np.zeros((4, 256, 128))
    fi = np.zeros((4, 128, 256))
    for p in range(4):
        for kk in range(128):
            fu[p, :, kk] = _fwd_col(4 * (kk // 2) + 256 * (kk % 2) + p)
            c = _out_row_time(p, kk)
            fi[p, kk, 0::2] = np.cos(_THETA * c) / T
            fi[p, kk, 1::2] = -np.sin(_THETA * c) / T
    val = -np.ones((3, 2, 128), dtype=np.int64)
    for i, pr in enumerate(A_PAIRS):
        for half in range(2):
            for jj in range(16):
                for hp in range(2):
                    lane = (8 * jj + 8 + hp + half + 2 * (i % 4)) % 128
                    val[i // 4, half, lane] = pr[half] + 8 * (jj + 16 * (1 - hp))
    tl = _build_tiles(val[0, 0], val[0, 1], val[1, 0], val[1, 1], val[2, 0], val[2, 1],
                      np.arange(128), np.where, np.roll)
    fg = np.zeros((len(G_LIST), 256, 128))
    for g, (ka, p, name) in enumerate(G_LIST):
        for m in range(1, T + 1):
            lag = T * ka + m
            if m % 4 != p or lag >= S:
                continue
            fg[g, :, int(np.where(tl[name] == _bf16_round_int(lag))[0][0])] += _fwd_col(m)
    fi2 = np.stack([fi[:, :, :128], fi[:, :, 128:]], axis=1)
    trig = np.stack([2 * np.cos(_THETA), 2 * np.sin(_THETA)])[:, :, None] * np.ones((1, 1, 128))
    return (_pack_rows(fu), _pack_rows(fi2), _pack_rows(fg), trig.astype(np.float32))


def _cmul(a, b):
    return (a[0] * b[0] - a[1] * b[1], a[0] * b[1] + a[1] * b[0])


def _csq(a):
    return (a[0] * a[0] - a[1] * a[1], (a[0] + a[0]) * a[1])


def _cadd(a, b):
    return (a[0] + b[0], a[1] + b[1])


def _csub(a, b):
    return (a[0] - b[0], a[1] - b[1])


def _add_i(a, b):
    return (a[0] - b[1], a[1] + b[0])


def _sub_i(a, b):
    return (a[0] + b[1], a[1] - b[0])


def _pack(a, b):
    return pltpu.bitcast(pltpu.pack_elementwise([a, b], packed_dtype=BF16), U32)


def _bf(x):
    return pltpu.bitcast(x, BF16)


def _dot(a, b):
    return jnp.dot(a, b, preferred_element_type=F32)


def _dot_t(a, b):
    return lax.dot_general(a, b, (((1,), (1,)), ((), ())), preferred_element_type=F32)


def _phi(t):
    return jnp.where(t > 0, t + 1.0, jnp.exp(t)) + 1e-6


def _kernel(x_h, wqkv_h, wo_h, u_h, are_h, aim_h, bre_h, bim_h, cre_h, cim_h, ldt_h, dsk_h,
            fu_h, fi_h, fg_h, trig_h, o_h,
            x_v, u_v, w3_v, wo_v, par_v, sm_v, fu_v, fi_v, fg_v, trig_v,
            zw_s, k0_s, pl_s, pw_s, pk_s, h_s, xu_s, q_s, ul_s, oa_s, ob_s,
            wkt_s, g_s, zacc_s, m_s, zm_s, sem, xsem, usem, asem, bsem):
    cps = dict(
        are=(are_h, par_v.at[0]), aim=(aim_h, par_v.at[1]), ldt=(ldt_h, sm_v.at[0]), dsk=(dsk_h, sm_v.at[1]),
        wk=(wqkv_h.at[:, 512:1024], w3_v.at[1]),
        bre=(bre_h, par_v.at[2]), bim=(bim_h, par_v.at[3]), cre=(cre_h, par_v.at[4]), cim=(cim_h, par_v.at[5]),
        fu=(fu_h, fu_v), fg=(fg_h, fg_v), trig=(trig_h, trig_v),
        wv=(wqkv_h.at[:, 1024:1536], w3_v.at[2]), wo=(wo_h, wo_v),
        wq=(wqkv_h.at[:, 0:512], w3_v.at[0]), fi=(fi_h, fi_v),
    )
    cps = {k: pltpu.make_async_copy(s_, d_, sem.at[i]) for i, (k, (s_, d_)) in enumerate(cps.items())}

    def xcp(j):
        r = pl.ds(pl.multiple_of(j * 512, 512), 512)
        return pltpu.make_async_copy(x_h.at[r, :], x_v.at[r, :], xsem.at[j])

    def ucp(c):
        return pltpu.make_async_copy(u_h.at[:, pl.ds(pl.multiple_of(c * 128, 128), 128)], u_v.at[c], usem.at[c])

    def acp(j):
        r = pl.ds(pl.multiple_of(j * 512, 512), 512)
        return pltpu.make_async_copy(oa_s.at[r, :], o_h.at[r, 0:512], asem.at[j])

    def bcp(c):
        return pltpu.make_async_copy(ob_s.at[c], o_h.at[:, pl.ds(pl.multiple_of(512 + c * 128, 128), 128)], bsem.at[c])

    for k in ('ldt', 'are', 'aim', 'dsk', 'bre', 'bim', 'cre', 'cim', 'wk'):
        cps[k].start()
    xcp(0).start()
    cps['fu'].start()
    ucp(0).start()
    for k in ('ldt', 'are', 'aim', 'dsk', 'bre', 'bim', 'cre', 'cim'):
        cps[k].wait()

    sub8 = lax.broadcasted_iota(jnp.int32, (8, 128), 0)
    lane8 = lax.broadcasted_iota(jnp.int32, (8, 128), 1)

    dt4 = jnp.exp(sm_v[0].astype(F32)).astype(BF16).astype(F32)
    dsk4 = sm_v[1].astype(F32)
    ones = jnp.ones((8, 128), BF16)
    for c in range(4):
        rows = slice(128 * c, 128 * c + 128)
        dtb = jnp.broadcast_to(dt4[c:c + 1], (128, 128)).T
        lr = dtb * par_v[0, rows].astype(F32)
        li = dtb * par_v[1, rows].astype(F32)
        mag = jnp.exp(lr)
        zw_s[0, rows] = mag * jnp.cos(li)
        zw_s[1, rows] = mag * jnp.sin(li)
        db = (dtb * par_v[2, rows].astype(F32), dtb * par_v[3, rows].astype(F32))
        w = _cmul((par_v[4, rows].astype(F32), par_v[5, rows].astype(F32)), db)
        zw_s[2, rows] = w[0]
        zw_s[3, rows] = w[1]
        k0_s[c] = _dot_t(ones, w[0].astype(BF16)) + dsk4[c:c + 1]
        if c == 1:
            cps['wk'].wait()
            wkt_s[...] = pltpu.bitcast(w3_v[1].T, U32)
    g_s[...] = jnp.zeros((512, 512), F32)
    zacc_s[...] = jnp.zeros((512, 128), F32)
    cps['fu'].wait()
    for j in range(1, 4):
        xcp(j).start()
        ucp(j).start()
    for k in ('fg', 'trig', 'wv', 'wo', 'wq', 'fi'):
        cps[k].start()

    perm_mask = (sub8 % 4) < 2
    slot = ((lane8 + 8 - (sub8 % 2)) % 8) // 2

    def perm(v):
        return jnp.where(perm_mask, pltpu.roll(v, 2, 0), pltpu.roll(v, 6, 0))

    def kgen_block(blk, sl):
        r = pl.multiple_of(blk * 8, 8)
        z1 = (zw_s[0, pl.ds(r, 8)], zw_s[1, pl.ds(r, 8)])
        w = (zw_s[2, pl.ds(r, 8)], zw_s[3, pl.ds(r, 8)])
        z2 = _csq(z1)
        z4 = _csq(z2)
        z8 = _csq(z4)
        W = [None] * 16
        W[1] = (perm(z8[0]), perm(z8[1]))
        W[2] = _csq(W[1])
        W[4] = _csq(W[2])
        W[8] = _csq(W[4])
        w16 = _csq(W[8])
        W[3] = _cmul(W[2], W[1])
        for j in (1, 2, 3):
            W[4 + j] = _cmul(W[4], W[j])
        pw_s[sl, 0, 0:8] = _pack(w16[0], jnp.ones((8, 128), F32))
        pw_s[sl, 1, 0:8] = _pack(w16[1], jnp.zeros((8, 128), F32))
        for j in range(1, 16):
            if W[j] is None:
                W[j] = _cmul(W[8], W[j - 8])
            hi = _cmul(W[j], w16)
            pw_s[sl, 0, 8 * j:8 * j + 8] = _pack(hi[0], W[j][0])
            pw_s[sl, 1, 8 * j:8 * j + 8] = _pack(hi[1], W[j][1])
        t = _csq(w16)
        z256 = (perm(t[0]), perm(t[1]))
        z512 = _csq(z256)
        z1024 = _csq(z512)
        Lt = {}
        Lt[1] = _cmul(w, z1)
        Lt[2] = _cmul(w, z2)
        Lt[3] = _cmul(Lt[1], z2)
        Lt[4] = _cmul(w, z4)
        for a in (1, 2, 3):
            Lt[4 + a] = _cmul(Lt[a], z4)
        Lt[8] = _cmul(w, z8)
        for a in (2, 4, 6, 8):
            Lt[256 + a] = _cmul(Lt[a], z256)
        for a in (4, 8, 260, 264):
            Lt[512 + a] = _cmul(Lt[a], z512)
        for a in (8, 264, 520, 776):
            Lt[1024 + a] = _cmul(Lt[a], z1024)
        for i, (a0, a1) in enumerate(A_PAIRS):
            pl_s[sl, 0, 8 * i:8 * i + 8] = _pack(Lt[a0][0], Lt[a1][0])
            pl_s[sl, 1, 8 * i:8 * i + 8] = _pack(Lt[a0][1], Lt[a1][1])
        os_ = []
        for e in range(2):
            os_.append(
                _dot_t(_bf(pl_s[sl, 0, pl.ds(e, 40, stride=2)]), _bf(pw_s[sl, 0, pl.ds(e, 64, stride=2)]))
                - _dot_t(_bf(pl_s[sl, 1, pl.ds(e, 40, stride=2)]), _bf(pw_s[sl, 1, pl.ds(e, 64, stride=2)])))
        o = _pack(os_[0], os_[1])
        rot = [pltpu.roll(o[8 * i:8 * i + 8], 2 * (i % 4) + 2, 1, stride=1, stride_axis=0)
               for i in range(10)]
        c01 = [jnp.where(slot == 0, rot[4 * c], rot[4 * c + 1]) for c in range(3)]
        c23 = [jnp.where(slot == 2, rot[4 * c + 2], rot[4 * c + 3]) for c in range(2)]
        pk_s[0, pl.ds(r, 8)] = jnp.where(slot < 2, c01[0], c23[0])
        pk_s[1, pl.ds(r, 8)] = jnp.where(slot < 2, c01[1], c23[1])
        pk_s[2, pl.ds(r, 8)] = c01[2]

    def cpos(m, rho):
        return (m[16 * rho:16 * rho + 8], m[16 * rho + 8:16 * rho + 16])

    def store_bins(ref, idx, rho, a, b, c, d_):
        xs = (_cadd(a, c), _sub_i(b, d_), _csub(a, c), _add_i(b, d_))
        for r_, v in enumerate(xs):
            ref[idx, r_, 16 * rho:16 * rho + 8] = v[0]
            ref[idx, r_, 16 * rho + 8:16 * rho + 16] = v[1]

    def hstage(c):
        r0 = c * 128
        lane = lax.broadcasted_iota(jnp.int32, (64, 128), 1)
        base = [pk_s[k, pl.ds(r0 + h, 64, stride=2)] for k in range(3) for h in range(2)]
        tl = _build_tiles(*base, lane, jnp.where, lambda v, s_: pltpu.roll(v, s_, 1))
        P = {}
        for g, (ka, p, name) in enumerate(G_LIST):
            P[(ka, p)] = _dot_t(_bf(fg_v[g]), _bf(tl[name]))
        for ka in range(4):
            for rho in range(16):
                p0, p2 = cpos(P[(ka, 0)], rho), cpos(P[(ka, 2)], rho)
                a, b = _cadd(p0, p2), _csub(p0, p2)
                if ka < 2:
                    p1, p3 = cpos(P[(ka, 1)], rho), cpos(P[(ka, 3)], rho)
                    store_bins(h_s, c * 4 + ka, rho, a, b, _cadd(p1, p3), _csub(p1, p3))
                else:
                    c2, s2 = trig_v[0, 8 * rho:8 * rho + 8], trig_v[1, 8 * rho:8 * rho + 8]
                    cc = (c2 * p2[0], c2 * p2[1])
                    ss = (s2 * p2[0], s2 * p2[1])
                    for r_, v in enumerate((_cadd(a, cc), _cadd(b, ss), _csub(a, cc), _csub(b, ss))):
                        h_s[c * 4 + ka, r_, 16 * rho:16 * rho + 8] = v[0]
                        h_s[c * 4 + ka, r_, 16 * rho + 8:16 * rho + 16] = v[1]

    def ustage(c):
        for j in range(4):
            v = pltpu.bitcast(u_v[c, 512 * j:512 * j + 512, :], U32)
            a, b = v[:128], v[128:]
            ul_s[j, 0] = (a & jnp.uint32(0xFFFF)) | (b << 16)
            ul_s[j, 1] = (a >> 16) | (b & jnp.uint32(0xFFFF0000))
            P = [_dot(_bf(fu_v[p]), _bf(ul_s[j, p % 2, pl.ds(p // 2, 64, stride=2)])) for p in range(4)]
            for rho in range(16):
                p0, p1, p2, p3 = [cpos(m, rho) for m in P]
                store_bins(xu_s, c * 4 + j, rho, _cadd(p0, p2), _csub(p0, p2), _cadd(p1, p3), _csub(p1, p3))

    def mac_pos(c, rho):
        r0 = rho * 16
        k0 = k0_s[c]
        Y = []
        for r_ in range(4):
            X = [(xu_s[c * 4 + j, r_, pl.ds(r0, 8)], xu_s[c * 4 + j, r_, pl.ds(r0 + 8, 8)]) for j in range(4)]
            H = [(h_s[c * 4 + j, r_, pl.ds(r0, 8)], h_s[c * 4 + j, r_, pl.ds(r0 + 8, 8)]) for j in range(4)]
            comb = _sub_i if rho >= 8 else _add_i
            G = [(H[0][0] + k0, H[0][1])] + [comb(H[k], H[k - 1]) for k in range(1, 4)]
            ys = []
            for i in range(4):
                acc = _cmul(G[0], X[i])
                for k in range(1, i + 1):
                    acc = _cadd(acc, _cmul(G[k], X[i - k]))
                ys.append(acc)
            Y.append(ys)
        q0 = rho * 8
        for i in range(4):
            e, f = _cadd(Y[0][i], Y[2][i]), _csub(Y[0][i], Y[2][i])
            g, h = _cadd(Y[1][i], Y[3][i]), _csub(Y[1][i], Y[3][i])
            for p, v in enumerate((_cadd(e, g), _add_i(f, h), _csub(e, g), _sub_i(f, h))):
                q_s[i, p, pl.ds(q0, 8)] = _pack(v[0], v[1])

    def inv_stage(c):
        even = (lax.broadcasted_iota(jnp.int32, (16, 8, 128), 1) % 2) == 0
        for i in range(4):
            y = [_dot(_bf(fi_v[p, 0]), _bf(q_s[i, p, 0:64])) + _dot(_bf(fi_v[p, 1]), _bf(q_s[i, p, 64:128]))
                 for p in range(4)]
            ev = _pack(y[0], y[1]).reshape(16, 8, 128)
            od = _pack(y[2], y[3]).reshape(16, 8, 128)
            v0 = jnp.where(even, ev, od)
            v1 = pltpu.roll(jnp.where(even, od, ev), 7, 1)
            v = jnp.stack([v0, v1], axis=1).reshape(256, 128)
            ob_s[c, 512 * i:512 * i + 512] = _bf(v)

    def kg_stage(j):
        xc = x_v[pl.ds(pl.multiple_of(j * 512, 512), 512), :]
        pk = _phi(_dot_t(_bf(wkt_s[...]), xc))
        zacc_s[...] += (pk[:, 0:128] + pk[:, 128:256]) + (pk[:, 256:384] + pk[:, 384:512])
        g_s[...] += _dot(pk.astype(BF16), xc)

    def m_stage():
        hm = (lax.broadcasted_iota(jnp.int32, (128, 128), 0) // 16) == (lax.broadcasted_iota(jnp.int32, (128, 128), 1) // 16)
        for g in range(4):
            rows = slice(128 * g, 128 * g + 128)
            kv = jnp.where(hm, _dot(g_s[rows].astype(BF16), w3_v[2, :, rows]), 0.0)
            m_s[64 * g:64 * g + 64] = pltpu.bitcast(_dot(kv.astype(BF16), wo_v[rows]).astype(BF16), U32)
            z = jnp.sum(zacc_s[rows], axis=1, keepdims=True)
            zm_s[g] = pltpu.bitcast(jnp.where(hm, z, 0.0).astype(BF16), U32)

    def q_stage(j):
        r = pl.ds(pl.multiple_of(j * 512, 512), 512)
        pq = _phi(_dot(x_v[r, :], w3_v[0]))
        pb = pq.astype(BF16)
        den = jnp.concatenate([_dot(pb[:, 128 * g:128 * g + 128], _bf(zm_s[g])) for g in range(4)], axis=1) + 1e-6
        o = (pq * pl.reciprocal(den, approx=True)).astype(BF16)
        oa_s[r, :] = _dot(o, _bf(m_s[...])).astype(BF16)

    def loop1(c, cr):
        xcp(c).wait()
        ucp(c).wait()
        for sl in range(16):
            kgen_block(c * 16 + sl, sl)
        kg_stage(c)
        ustage(c)
        return cr
    lax.fori_loop(0, 4, loop1, 0)

    for k in ('fg', 'trig', 'wv', 'wo', 'wq', 'fi'):
        cps[k].wait()
    m_stage()
    for c in range(4):
        hstage(c)

    def loop2(c, cr):
        for rho in range(16):
            mac_pos(c, rho)
        q_stage(c)
        inv_stage(c)
        acp(c).start()
        bcp(c).start()
        return cr
    lax.fori_loop(0, 4, loop2, 0)
    for c in range(4):
        acp(c).wait()
        bcp(c).wait()


@jax.jit
def pallas_concat_heads__linear_attn_block__ssm_conv_s4__prompt_kernel(
    A_x, A_wqkv, A_wo, B_u, B_A_re, B_A_im, B_B_re, B_B_im, B_C_re, B_C_im, B_log_dt, B_Dskip,
):
    fu, fi, fg, trig = _tables()
    V = pltpu.VMEM
    scratch = [
        V((S, D), BF16), V((4, S, 128), BF16), V((3, D, D), BF16), V((D, D), BF16),
        V((6, D, 128), BF16), V((2, 4, 128), BF16),
        V(fu.shape, U32), V(fi.shape, U32), V(fg.shape, U32), V(trig.shape, F32),
        V((4, D, 128), F32), V((4, 8, 128), F32),
        V((16, 2, 80, 128), U32), V((16, 2, 128, 128), U32), V((3, D, 128), U32),
        V((16, 4, 256, 128), F32), V((16, 4, 256, 128), F32), V((4, 4, 128, 128), U32),
        V((4, 2, 128, 128), U32), V((S, D), BF16), V((4, S, 128), BF16),
        V((256, D), U32), V((D, D), F32), V((D, 128), F32), V((256, D), U32), V((4, 64, 128), U32),
        pltpu.SemaphoreType.DMA((16,)), pltpu.SemaphoreType.DMA((4,)), pltpu.SemaphoreType.DMA((4,)),
        pltpu.SemaphoreType.DMA((4,)), pltpu.SemaphoreType.DMA((4,)),
    ]
    out = pl.pallas_call(
        _kernel,
        out_shape=jax.ShapeDtypeStruct((S, 2 * D), BF16),
        in_specs=[pl.BlockSpec(memory_space=pl.ANY)] * 16,
        out_specs=pl.BlockSpec(memory_space=pl.ANY),
        scratch_shapes=scratch,
        compiler_params=pltpu.CompilerParams(vmem_limit_bytes=100 * 1024 * 1024),
    )(A_x.reshape(S, D), A_wqkv, A_wo, B_u.reshape(S, D), B_A_re, B_A_im, B_B_re, B_B_im,
      B_C_re, B_C_im, B_log_dt.reshape(4, 128), B_Dskip.reshape(4, 128),
      jnp.asarray(fu), jnp.asarray(fi), jnp.asarray(fg), jnp.asarray(trig))
    return out.reshape(1, S, 2 * D)
```

```python
import functools
import os
import contextlib

import jax
import jax.numpy as jnp
import numpy as np
from jax import lax
import jax.experimental.pallas as pl
import jax.experimental.pallas.tpu as pltpu

def _scope(name):
    return jax.named_scope(name) if os.environ.get('KSCOPES') else contextlib.nullcontext()


WAR = not os.environ.get('CONS')
F32 = jnp.float32
BF16 = jnp.bfloat16
U32 = jnp.uint32

S = 2048
D = 512
T = 512


def _bf16_bits(x):
    u = np.ascontiguousarray(x, dtype=np.float32).view(np.uint32).astype(np.uint64)
    return (((u + 0x7FFF + ((u >> 16) & 1)) >> 16) & 0xFFFF).astype(np.uint32)


def _bf16_round_int(l):
    return int((_bf16_bits(np.array([l], np.float32)) << 16).view(np.float32)[0])


def _pack_rows(m):
    b = _bf16_bits(m)
    return (b[..., 0::2, :] | (b[..., 1::2, :] << 16)).astype(np.uint32)


_F_OF_ROW = np.array([2 * (8 * ((r // 8) % 8) + r % 8) + (r // 64) for r in range(128)])
_THETA = 2 * np.pi * (_F_OF_ROW + 0.5) / (2 * T)


def _fwd_col(m):
    c = np.cos(_THETA * m).reshape(16, 8)
    s = -np.sin(_THETA * m).reshape(16, 8)
    return np.concatenate([c, s], axis=1).reshape(256)


def _out_row_time(p, r):
    t2, s = r // 8, r % 8
    if (s % 2 == 0) == (p < 2):
        w, v = s, 0
    else:
        w, v = (s - 1) % 8, 1
    return 32 * t2 + 16 * v + 2 * w + (p % 2)


def _in_row_time(p, kk):
    q, h = kk // 2, kk % 2
    t, s = q // 8, q % 8
    if (s % 2 == 0) == (p < 2):
        w = 8 * t + s
    else:
        w = 64 + 8 * t + (s - 1) % 8
    return 256 * h + 2 * w + (p % 2)


A_PAIRS = ((4, 2), (8, 6), (260, 258), (264, 262),
           (1, 516), (5, 520), (1544, 772), (1800, 776),
           (3, 1032), (7, 1288))
G_LIST = ((0, 0, 'TA0'), (0, 1, 'TA1'), (0, 2, 'TA2'), (0, 3, 'TA3'),
          (1, 0, 'TB'), (1, 3, 'TB'), (1, 1, 'TB1'), (1, 2, 'TB2'),
          (2, 0, 'TC'), (2, 2, 'TC'), (3, 0, 'TD'), (3, 2, 'TD'))
LANE_512, LANE_1024 = 6, 7


def _build_tiles(x1, y1, x2, y2, x3, y3, lane, where, roll):
    low_x = (lane % 8) < 4
    low_y = ((lane + 7) % 8) < 4
    return dict(
        TA0=x1,
        TA1=where(lane == LANE_512, roll(x1, 4), where(low_x, x2, x1)),
        TA2=y1,
        TA3=where(low_x, x3, x1),
        TB=y2,
        TB1=where(lane == LANE_1024, roll(x1, 1), y2),
        TB2=where(lane == LANE_512, x1, y2),
        TC=where(low_y, y3, y2),
        TD=where(low_x, y3, x2),
    )


@functools.lru_cache(maxsize=None)
def _tables():
    fu = np.zeros((4, 256, 128))
    fi = np.zeros((4, 128, 256))
    for p in range(4):
        for kk in range(128):
            fu[p, :, kk] = _fwd_col(_in_row_time(p, kk))
            c = _out_row_time(p, kk)
            fi[p, kk, 0::2] = np.cos(_THETA * c) / T
            fi[p, kk, 1::2] = -np.sin(_THETA * c) / T
    val = -np.ones((3, 2, 128), dtype=np.int64)
    for i, pr in enumerate(A_PAIRS):
        for half in range(2):
            for jj in range(16):
                for hp in range(2):
                    lane = (8 * jj + 8 + hp + half + 2 * (i % 4)) % 128
                    val[i // 4, half, lane] = pr[half] + 8 * (jj + 16 * (1 - hp))
    tl = _build_tiles(val[0, 0], val[0, 1], val[1, 0], val[1, 1], val[2, 0], val[2, 1],
                      np.arange(128), np.where, np.roll)
    fg = np.zeros((len(G_LIST), 256, 128))
    for g, (ka, p, name) in enumerate(G_LIST):
        for m in range(1, T + 1):
            lag = T * ka + m
            if m % 4 != p or lag >= S:
                continue
            fg[g, :, int(np.where(tl[name] == _bf16_round_int(lag))[0][0])] += _fwd_col(m)
    fi2 = np.stack([fi[:, :, :128], fi[:, :, 128:]], axis=1)
    trig = np.stack([2 * np.cos(_THETA), 2 * np.sin(_THETA)])[:, :, None] * np.ones((1, 1, 128))
    return (_pack_rows(fu), _pack_rows(fi2), _pack_rows(fg), trig.astype(np.float32))


def _cmul(a, b):
    return (a[0] * b[0] - a[1] * b[1], a[0] * b[1] + a[1] * b[0])


def _csq(a):
    return (a[0] * a[0] - a[1] * a[1], (a[0] + a[0]) * a[1])


def _cadd(a, b):
    return (a[0] + b[0], a[1] + b[1])


def _csub(a, b):
    return (a[0] - b[0], a[1] - b[1])


def _add_i(a, b):
    return (a[0] - b[1], a[1] + b[0])


def _sub_i(a, b):
    return (a[0] + b[1], a[1] - b[0])


def _pack(a, b):
    return pltpu.bitcast(pltpu.pack_elementwise([a, b], packed_dtype=BF16), U32)


def _bf(x):
    return pltpu.bitcast(x, BF16)


def _dot(a, b):
    return jnp.dot(a, b, preferred_element_type=F32)


def _dot_t(a, b):
    return lax.dot_general(a, b, (((1,), (1,)), ((), ())), preferred_element_type=F32)


def _mo(i, n):
    return i if isinstance(i, int) else pl.multiple_of(i, n)


def _phi(t):
    return jnp.where(t > 0, t + 1.0, jnp.exp(t)) + 1e-6


NT, LAG = int(os.environ.get('NT', 12)), 4
NK = NT - LAG


def _kernel(x_h, wqkv_h, wo_h, u_h, are_h, aim_h, bre_h, bim_h, cre_h, cim_h, ldt_h, dsk_h,
            fu_h, fi_h, fg_h, trig_h, o_h,
            x_v, u_v, wq_v, wk_v, wv_v, wo_v, par_v, sm_v, fu_v, fi_v, fg_v, trig_v,
            wre_s, dt_s, z_s, pl_s, pw_s, pk_s, h_s, xu_s, oa_s, ob_s,
            wkt_s, wqt_s, g_s, zacc_s, m_s, zb_s, t0_s, t1_s, o0_s, o1_s, o2_s, o3_s, q0_s, q1_s, q2_s, q3_s, sem, xsem, osem):
    def tiled(src, col0, dst, sm, rows=None):
        r = slice(None) if rows is None else rows
        return [pltpu.make_async_copy(src.at[r, col0 + 128 * m:col0 + 128 * m + 128],
                                      dst.bitcast(BF16).at[m, r, :], sm) for m in range(4)]

    def one(src, dst, sm):
        return [pltpu.make_async_copy(src, dst, sm)]

    pars = (are_h, aim_h, bre_h, bim_h, cre_h, cim_h)

    def pcps(c, which=range(6), sm=None):
        r = pl.ds(_mo(c * 128, 128), 128)
        sm = xsem.at[c - 1] if sm is None else sm
        return [pltpu.make_async_copy(pars[i].at[r, :], par_v.at[i, r, :], sm) for i in which]

    def xcps(j):
        return tiled(x_h, 0, x_v, xsem.at[j], pl.ds(_mo(j * 512, 512), 512))

    last = xsem.at[3]
    cps = dict(
        ldt=one(ldt_h, sm_v.at[0], sem.at[0]), p0=pcps(0, sm=sem.at[1]), wk=tiled(wqkv_h, 512, wk_v, sem.at[2]),
        dsk=one(dsk_h, sm_v.at[1], last), fu=one(fu_h, fu_v, last), fg=one(fg_h, fg_v, last),
        trig=one(trig_h, trig_v, last), fi=one(fi_h, fi_v, last), u=tiled(u_h, 0, u_v, last),
        wv=tiled(wqkv_h, 1024, wv_v, last), wq=tiled(wqkv_h, 0, wq_v, last), wo=tiled(wo_h, 0, wo_v, last),
        p1=pcps(1), p2=pcps(2), p3=pcps(3), x0=xcps(0), x1=xcps(1), x2=xcps(2), x3=xcps(3),
    )

    def wide(ref, rows):
        return jnp.concatenate([ref[m, rows] for m in range(4)], axis=1)

    def acp(j, h):
        r = pl.ds(_mo(j * 512 + h * 256, 256), 256)
        return pltpu.make_async_copy(oa_s.at[r, :], o_h.at[r, 0:512], osem)

    def bcp(c, i):
        r = pl.ds(512 * i, 512)
        return pltpu.make_async_copy(ob_s.bitcast(BF16).at[i, c], o_h.at[r, pl.ds(_mo(512 + c * 128, 128), 128)], osem)

    sub8 = lax.broadcasted_iota(jnp.int32, (8, 128), 0)
    lane8 = lax.broadcasted_iota(jnp.int32, (8, 128), 1)

    def dt_stage():
        dt4 = jnp.exp(sm_v[0].astype(F32)).astype(BF16).astype(F32)
        for c in range(4):
            dt_s[128 * c:128 * c + 128] = jnp.broadcast_to(dt4[c:c + 1], (128, 128)).T

    perm_mask = (sub8 % 4) < 2
    slot = ((lane8 + 8 - (sub8 % 2)) % 8) // 2

    def perm(v):
        return jnp.where(perm_mask, pltpu.roll(v, 2, 0), pltpu.roll(v, 6, 0))

    def z_of(rows):
        dtb = dt_s[rows]
        li = dtb * par_v[1, rows].astype(F32)
        mag = jnp.exp(dtb * par_v[0, rows].astype(F32))
        return (mag * jnp.cos(li), mag * jnp.sin(li))

    def tab_block(blk, sl, z1=None):
        rows = pl.ds(_mo(8 * blk, 8), 8)
        dtb = dt_s[rows]
        if z1 is None:
            z1 = z_of(rows)
        db = (dtb * par_v[2, rows].astype(F32), dtb * par_v[3, rows].astype(F32))
        w = _cmul((par_v[4, rows].astype(F32), par_v[5, rows].astype(F32)), db)
        wre_s[rows] = w[0]
        z2 = _csq(z1)
        z4 = _csq(z2)
        z8 = _csq(z4)
        W = [None] * 16
        W[1] = (perm(z8[0]), perm(z8[1]))
        W[2] = _csq(W[1])
        W[4] = _csq(W[2])
        W[8] = _csq(W[4])
        w16 = _csq(W[8])
        W[3] = _cmul(W[2], W[1])
        for j in (1, 2, 3):
            W[4 + j] = _cmul(W[4], W[j])
        pw_s[sl, 0, 0:8] = _pack(w16[0], jnp.ones((8, 128), F32))
        pw_s[sl, 1, 0:8] = _pack(w16[1], jnp.zeros((8, 128), F32))
        for j in range(1, 16):
            if W[j] is None:
                W[j] = _cmul(W[8], W[j - 8])
            hi = _cmul(W[j], w16)
            pw_s[sl, 0, 8 * j:8 * j + 8] = _pack(hi[0], W[j][0])
            pw_s[sl, 1, 8 * j:8 * j + 8] = _pack(hi[1], W[j][1])
        t = _csq(w16)
        z256 = (perm(t[0]), perm(t[1]))
        z512 = _csq(z256)
        z1024 = _csq(z512)
        Lt = {}
        Lt[1] = _cmul(w, z1)
        Lt[2] = _cmul(w, z2)
        Lt[3] = _cmul(Lt[1], z2)
        Lt[4] = _cmul(w, z4)
        for a in (1, 2, 3):
            Lt[4 + a] = _cmul(Lt[a], z4)
        Lt[8] = _cmul(w, z8)
        for a in (2, 4, 6, 8):
            Lt[256 + a] = _cmul(Lt[a], z256)
        for a in (4, 8, 260, 264):
            Lt[512 + a] = _cmul(Lt[a], z512)
        for a in (8, 264, 520, 776):
            Lt[1024 + a] = _cmul(Lt[a], z1024)
        for i, (a0, a1) in enumerate(A_PAIRS):
            pl_s[sl, 0, 8 * i:8 * i + 8] = _pack(Lt[a0][0], Lt[a1][0])
            pl_s[sl, 1, 8 * i:8 * i + 8] = _pack(Lt[a0][1], Lt[a1][1])

    def km_block(blk, sl):
        r = _mo(blk * 8, 8)
        os_ = []
        for e in range(2):
            os_.append(
                _dot_t(_bf(pl_s[sl, 0, pl.ds(e, 40, stride=2)]), _bf(pw_s[sl, 0, pl.ds(e, 64, stride=2)]))
                - _dot_t(_bf(pl_s[sl, 1, pl.ds(e, 40, stride=2)]), _bf(pw_s[sl, 1, pl.ds(e, 64, stride=2)])))
        o = _pack(os_[0], os_[1])
        rot = [pltpu.roll(o[8 * i:8 * i + 8], 2 * (i % 4) + 2, 1, stride=1, stride_axis=0)
               for i in range(10)]
        c01 = [jnp.where(slot == 0, rot[4 * c], rot[4 * c + 1]) for c in range(3)]
        c23 = [jnp.where(slot == 2, rot[4 * c + 2], rot[4 * c + 3]) for c in range(2)]
        pk_s[0, pl.ds(r, 8)] = jnp.where(slot < 2, c01[0], c23[0])
        pk_s[1, pl.ds(r, 8)] = jnp.where(slot < 2, c01[1], c23[1])
        pk_s[2, pl.ds(r, 8)] = c01[2]

    def cpos(m, rho):
        return (m[16 * rho:16 * rho + 8], m[16 * rho + 8:16 * rho + 16])

    def store4(ref, idx, rho, xs):
        for r_, v in enumerate(xs):
            ref[idx, r_, 16 * rho:16 * rho + 8] = v[0]
            ref[idx, r_, 16 * rho + 8:16 * rho + 16] = v[1]

    def bfly(p0, p1, p2, p3):
        a, b, c, d_ = _cadd(p0, p2), _csub(p0, p2), _cadd(p1, p3), _csub(p1, p3)
        return (_cadd(a, c), _sub_i(b, d_), _csub(a, c), _add_i(b, d_))

    def h_pieces(c):
        r0 = c * 128
        tl = {}

        def piece(kas):
            def f():
                if not tl:
                    lane = lax.broadcasted_iota(jnp.int32, (64, 128), 1)
                    base = [pk_s[k, pl.ds(r0 + h, 64, stride=2)] for k in range(3) for h in range(2)]
                    tl.update(_build_tiles(*base, lane, jnp.where, lambda v, s_: pltpu.roll(v, s_, 1)))
                if 0 in kas:
                    k0 = (_dot_t(jnp.ones((8, 128), BF16), wre_s[r0:r0 + 128].astype(BF16))
                          + sm_v[1].astype(F32)[c:c + 1])
                P = {}
                for g, (ka, p, name) in enumerate(G_LIST):
                    if ka in kas:
                        P[(ka, p)] = _dot_t(_bf(fg_v[g]), _bf(tl[name]))
                for ka in kas:
                    for rho in range(16):
                        p0, p2 = cpos(P[(ka, 0)], rho), cpos(P[(ka, 2)], rho)
                        if ka == 0:
                            p0 = (p0[0] + k0, p0[1])
                        if ka < 2:
                            xs = bfly(p0, cpos(P[(ka, 1)], rho), p2, cpos(P[(ka, 3)], rho))
                        else:
                            a, b = _cadd(p0, p2), _csub(p0, p2)
                            c2, s2 = trig_v[0, 8 * rho:8 * rho + 8], trig_v[1, 8 * rho:8 * rho + 8]
                            cc = (c2 * p2[0], c2 * p2[1])
                            ss = (s2 * p2[0], s2 * p2[1])
                            xs = (_cadd(a, cc), _cadd(b, ss), _csub(a, cc), _csub(b, ss))
                        store4(h_s, c * 4 + ka, rho, xs)
            return f
        return [piece((0,)), piece((1,)), piece((2, 3))]

    def u_piece(c, j):
        even = (lax.broadcasted_iota(jnp.int32, (8, 8, 128), 1) % 2) == 0
        a = u_v[c, 256 * j:256 * j + 128]
        b = u_v[c, 256 * j + 128:256 * j + 256]
        ph = [None] * 4
        for h, m in enumerate(((a & jnp.uint32(0xFFFF)) | (b << 16), (a >> 16) | (b & jnp.uint32(0xFFFF0000)))):
            m1 = m[:64].reshape(8, 8, 128)
            m2 = pltpu.roll(m[64:].reshape(8, 8, 128), 1, 1)
            ph[h] = jnp.where(even, m1, m2).reshape(64, 128)
            ph[2 + h] = jnp.where(even, m2, m1).reshape(64, 128)
        P = [_dot(_bf(fu_v[p]), _bf(ph[p])) for p in range(4)]
        for rho in range(16):
            store4(xu_s, c * 4 + j, rho, bfly(*[cpos(m, rho) for m in P]))

    def mac(c, i, rho):
        r0 = rho * 16
        comb = _sub_i if rho >= 8 else _add_i
        Y = []
        for r_ in range(4):
            acc, hprev = None, None
            for k in range(i + 1):
                hk = (h_s[c * 4 + k, r_, r0:r0 + 8], h_s[c * 4 + k, r_, r0 + 8:r0 + 16])
                xk = (xu_s[c * 4 + i - k, r_, r0:r0 + 8], xu_s[c * 4 + i - k, r_, r0 + 8:r0 + 16])
                t = _cmul(hk if k == 0 else comb(hk, hprev), xk)
                acc = t if k == 0 else _cadd(acc, t)
                hprev = hk
            Y.append(acc)
        e, f = _cadd(Y[0], Y[2]), _csub(Y[0], Y[2])
        g, h = _cadd(Y[1], Y[3]), _csub(Y[1], Y[3])
        return [_pack(v[0], v[1]) for v in (_cadd(e, g), _add_i(f, h), _csub(e, g), _sub_i(f, h))]

    def inv_piece(c, i, qs, fi):
        y = [_dot(_bf(fi[p][0]), _bf(jnp.concatenate([qs[rho][p] for rho in range(8)], axis=0)))
             + _dot(_bf(fi[p][1]), _bf(jnp.concatenate([qs[rho][p] for rho in range(8, 16)], axis=0)))
             for p in range(4)]
        even = (lax.broadcasted_iota(jnp.int32, (16, 8, 128), 1) % 2) == 0
        ev = _pack(y[0], y[1]).reshape(16, 8, 128)
        od = _pack(y[2], y[3]).reshape(16, 8, 128)
        v0 = jnp.where(even, ev, od)
        v1 = pltpu.roll(jnp.where(even, od, ev), 7, 1)
        ob_s[i, c] = jnp.stack([v0, v1], axis=1).reshape(256, 128)
        bcp(c, i).start()

    def _pk16(v):
        if v.shape[1] > 128:
            return pltpu.bitcast(v.astype(BF16), U32)
        n = v.shape[0] // 32
        v4 = v.reshape(n, 2, 16, 128)
        w = jnp.concatenate([v4[:, 0], v4[:, 1]], axis=2).reshape(n * 16, 256)
        w = pltpu.bitcast(w.astype(BF16), U32).reshape(n, 8, 256)
        return jnp.stack([w[:, :, :128], w[:, :, 128:]], axis=1).reshape(n * 16, 128)

    def kg_pieces(j, j2):
        r0 = _mo(j * 256, 256)
        ts = (t0_s, t1_s)

        def kt_piece(n, h):
            def f():
                xt = wide(x_v, pl.ds(r0 + 64 * n, 64))
                pk = _phi(_dot_t(_bf(wkt_s[128 * h:128 * h + 128]), _bf(xt)))
                p3 = pk.reshape(16, 2, 8, 128)
                ts[h][j, :, 128 * n:128 * n + 128] = _pack(p3[:, 0], p3[:, 1]).reshape(128, 128)
                zacc_s[n, 256 * h:256 * h + 256] += pk
            return f

        def g_piece(n, h):
            def f():
                cols = slice(128 * n, 128 * n + 128)
                g_s[256 * h:256 * h + 256, cols] += _dot(_bf(ts[h][j2]), _bf(x_v[n, pl.ds(r0, 256)]))
            return f
        return ([kt_piece(n, 0) for n in range(4)] + [kt_piece(n, 1) for n in range(4)]
                + [g_piece(n, 0) for n in range(4)] + [g_piece(n, 1) for n in range(4)])

    def m_pieces():
        kvs = {}

        def hmask():
            return ((lax.broadcasted_iota(jnp.int32, (128, 128), 0) // 16)
                    == (lax.broadcasted_iota(jnp.int32, (128, 128), 1) // 16))

        def kv_piece(gs):
            def f():
                for g in gs:
                    rows = slice(128 * g, 128 * g + 128)
                    kv = _dot(g_s[rows].astype(BF16), _bf(wv_v[g]))
                    kvs[g] = jnp.where(hmask(), kv, 0.0).astype(BF16)
                    zs = (zacc_s[0, rows] + zacc_s[1, rows]) + (zacc_s[2, rows] + zacc_s[3, rows])
                    z = jnp.sum(zs, axis=1, keepdims=True)
                    zb_s[rows] = jnp.broadcast_to(z, (128, 128))
            return f

        def mm_piece(gs):
            def f():
                for g in gs:
                    m_s[64 * g:64 * g + 64] = _pk16(_dot(kvs[g], _bf(wide(wo_v, slice(64 * g, 64 * g + 64)))))
            return f
        return [kv_piece((0, 1)), kv_piece((2, 3)), mm_piece((0, 1)), mm_piece((2, 3))]

    def phase2(b, b2):
        r0 = _mo(b * 256, 256)
        os_ = (o0_s, o1_s, o2_s, o3_s)
        tile = [(i + b) % 4 for i in range(4)]
        qs = {i: {} for i in range(4)}
        todo = [(i, rho) for i in range(4) for rho in range(16)]

        q_s = (q0_s, q1_s, q2_s, q3_s)

        def domac(i, rho):
            for p, v in enumerate(mac(tile[i], i, rho)):
                q_s[i][0, p, 8 * rho:8 * rho + 8] = v

        def pin(cols, n):
            if not n:
                return cols
            never = dt_s[0:8] < -1.0
            nv = cols[0].shape[0] // 8
            rows = [[w[8 * t:8 * t + 8] for t in range(nv)] for w in cols]
            for k in range(n):
                i, rho = todo.pop(0)
                if WAR:
                    t = (k * nv) // n
                    for p in range(4):
                        rows[p][t] = jnp.where(never, q_s[i][0, p, 8 * rho:8 * rho + 8], rows[p][t])
                    domac(i, rho)
                    continue
                qs[i][rho] = mac(tile[i], i, rho)
                t = ((2 * k + 1) * nv) // (2 * n)
                for p in range(4):
                    rows[p][t] = jnp.where(never, qs[i][rho][p], rows[p][t])
            return [jnp.concatenate(r, axis=0) for r in rows]

        def split(w):
            return [w[:, 128 * m:128 * m + 128] for m in range(4)]

        def q_piece(n, h, k):
            wl = jnp.concatenate(pin(split(wqt_s[128 * h:128 * h + 128]), k), axis=1)
            pq = _phi(_dot_t(_bf(wl), _bf(wide(x_v, pl.ds(r0 + 64 * n, 64)))))
            t = (pq * zb_s[256 * h:256 * h + 256]).reshape(16, 2, 8, 128)
            den = t[:, 0] + t[:, 1]
            for sh in (4, 2, 1):
                den = den + pltpu.roll(den, sh, 1)
            rec = pl.reciprocal(den + 1e-6, approx=True)
            p3 = pq.reshape(16, 2, 8, 128)
            ot = _pack(p3[:, 0] * rec, p3[:, 1] * rec).reshape(128, 128)
            os_[n][0, :, 256 * h:256 * h + 256] = pltpu.bitcast(_bf(ot).T, U32)

        def out_piece(n, m, k):
            ol = split(os_[n][b2 - b])
            r = [_dot(_bf(jnp.concatenate(pin(ol, kk), axis=1)), _bf(m_s[:, 128 * mm:128 * mm + 128]))
                 for mm, kk in ((2 * m, k // 2), (2 * m + 1, k - k // 2))]
            oa_s[pl.ds(2 * r0 + 128 * n, 128), 256 * m:256 * m + 256] = jnp.concatenate(r, axis=1).astype(BF16)
            if m == 1 and n % 2 == 1:
                acp(b, n // 2).start()

        def inv(i, k):
            while todo and todo[0][0] == i:
                _, rho = todo.pop(0)
                qs[i][rho] = mac(tile[i], i, rho)
            if WAR:
                for rho in range(16):
                    if rho not in qs[i]:
                        qs[i][rho] = [q_s[i][b2 - b, p, 8 * rho:8 * rho + 8] for p in range(4)]
            k1 = k // 2
            f01 = pin([fi_v[0, 0], fi_v[0, 1], fi_v[1, 0], fi_v[1, 1]], k1)
            f23 = pin([fi_v[2, 0], fi_v[2, 1], fi_v[3, 0], fi_v[3, 1]], k - k1)
            inv_piece(tile[i], i, qs[i], [f01[0:2], f01[2:4], f23[0:2], f23[2:4]])

        q_piece(0, 0, 6)
        q_piece(0, 1, 4)
        q_piece(1, 0, 4)
        q_piece(1, 1, 3)
        out_piece(0, 0, 4)
        inv(0, 5)
        out_piece(0, 1, 5)
        q_piece(2, 0, 3)
        q_piece(2, 1, 1)
        inv(1, 2)
        out_piece(1, 0, 4)
        out_piece(1, 1, 4)
        q_piece(3, 0, 3)
        q_piece(3, 1, 1)
        out_piece(2, 0, 2)
        inv(2, 3)
        out_piece(2, 1, 4)
        out_piece(3, 0, 3)
        out_piece(3, 1, 3)
        inv(3, 0)
        assert not todo

    def start(*names):
        for k in names:
            for cp in cps[k]:
                cp.start()

    def wait(*names):
        for k in names:
            for cp in cps[k]:
                cp.wait()

    start('ldt', 'p0', 'wk')
    with _scope("init"):
        g_s[...] = jnp.zeros((512, 512), F32)
        zacc_s[...] = jnp.zeros((4, 512, 128), F32)
    with _scope("wait_ldt"):
        wait('ldt')
    with _scope("dt"):
        dt_stage()
        for q in (q0_s, q1_s, q2_s, q3_s):
            q[0] = jnp.zeros((4, 128, 128), U32)
    with _scope("wait_par"):
        wait('p0')
    start('x0', 'p1')

    def zs(g):
        rows = pl.ds(_mo(8 * g, 8), 8)
        return (z_s[0, rows], z_s[1, rows])

    def z_rows(r0, n):
        rows = pl.ds(_mo(r0, 8), n)
        z = z_of(rows)
        z_s[0, rows] = z[0]
        z_s[1, rows] = z[1]

    PV = os.environ.get('PV', 'a')
    if PV == 'a':
        with _scope("pro1"):
            def zloop(t, cr):
                z_rows(t * 4 * NK, 4 * NK)
                for k in range(2):
                    tab_block(NK + 2 * t + k, 2 * t + k)
                return cr
            lax.fori_loop(0, 2, zloop, 0)
        with _scope("wait_wk"):
            wait('wk')
        with _scope("pro2"):
            for m in range(4):
                wkt_s[64 * m:64 * m + 64] = pltpu.bitcast(_bf(wk_v[m]).T, U32)
            for g in range(NK):
                tab_block(g, g + LAG, zs(g))
                km_block(g, g + LAG)
    else:
        with _scope("pro0"):
            z_rows(32, 48)
            for g in range(LAG):
                tab_block(g, g)

        def kt4(t, cr, z=True):
            for k in range(LAG):
                km_block(LAG * t + k, k)
                tab_block(LAG * (t + 1) + k, k, zs(LAG * (t + 1) + k))
            if z:
                z_rows(80 + t * 16, 32)
            return cr
        with _scope("pro1"):
            lax.fori_loop(0, 2, kt4, 0)
        with _scope("wait_wk"):
            wait('wk')
        with _scope("pro2"):
            for m in range(4):
                wkt_s[64 * m:64 * m + 64] = pltpu.bitcast(_bf(wk_v[m]).T, U32)
            kt4(2, 0, False)

    plan = [('x1', 'p2', 'dsk', 'fg', 'trig', 'fu'), ('x2', 'p3', 'u'), ('x3', 'wv', 'wo', 'wq', 'fi')]

    def loop1(c, cr):
        with _scope("wait_x"):
            for cp in xcps(c) + pcps(c + 1):
                cp.wait()
        with _scope("loop1"):
            for sl, f in enumerate(kg_pieces(c, cr)):
                km_block(NK + c * 16 + sl, sl % LAG)
                tab_block(NT + c * 16 + sl, sl % LAG)
                f()
        for k in range(2):
            pl.when(c == k)(functools.partial(start, *plan[k + 1]))
        return cr + 1
    start(*plan[0])
    three = lax.fori_loop(0, 3, loop1, 0)

    with _scope("wait_w"):
        wait('x3', 'dsk', 'fg', 'trig', 'fu', 'u', 'wv', 'wo', 'wq', 'fi')
    with _scope("mid"):
        for m in range(4):
            wqt_s[64 * m:64 * m + 64] = pltpu.bitcast(_bf(wq_v[m]).T, U32)
        hp = [f for c in range(4) for f in h_pieces(c)]
        up = [functools.partial(u_piece, c, j) for c in range(4) for j in range(4)]
        for sl, f in enumerate(kg_pieces(3, three)):
            if NK + 48 + sl < 64:
                km_block(NK + 48 + sl, sl % LAG)
            if NT + 48 + sl < 64:
                tab_block(NT + 48 + sl, sl % LAG)
            f()
            if NT + 48 + sl >= 64:
                (hp or up).pop(0)()
        up = hp + up
        for f in m_pieces():
            up.pop(0)()
            f()
        for f in up:
            f()

    def loop2(b, cr):
        with _scope("loop2"):
            phase2(b, cr)
        return cr + 1
    lax.fori_loop(0, 4, loop2, 0)
    with _scope("wait_out"):
        for c in range(4):
            for h in range(2):
                acp(c, h).wait()
            for i in range(4):
                bcp(c, i).wait()


@jax.jit
def pallas_concat_heads__linear_attn_block__ssm_conv_s4__prompt_kernel(
    A_x, A_wqkv, A_wo, B_u, B_A_re, B_A_im, B_B_re, B_B_im, B_C_re, B_C_im, B_log_dt, B_Dskip,
):
    fu, fi, fg, trig = _tables()
    V = pltpu.VMEM
    DMA = pltpu.SemaphoreType.DMA
    W = V((D // 2, D), U32)
    W4 = V((4, D // 2, 128), U32)
    H = V((4, 128, D), U32)
    Q = V((2, 4, 128, 128), U32)
    O = V((2, 64, D), U32)
    scratch = [
        V((4, S // 2, 128), U32), V((4, S // 2, 128), U32), W4, W4, W4, W4,
        V((6, D, 128), BF16), V((2, 4, 128), BF16),
        V(fu.shape, U32), V(fi.shape, U32), V(fg.shape, U32), V(trig.shape, F32),
        V((D, 128), F32), V((D, 128), F32), V((2, 128, 128), F32),
        V((NT, 2, 80, 128), U32), V((NT, 2, 128, 128), U32), V((3, D, 128), U32),
        V((16, 4, 256, 128), F32), V((16, 4, 256, 128), F32),
        V((S, D), BF16), V((4, 4, 256, 128), U32),
        W, W, V((D, D), F32), V((4, D, 128), F32), W, V((D, 128), F32), H, H, O, O, O, O, Q, Q, Q, Q,
        DMA((3,)), DMA((4,)), DMA(()),
    ]
    out = pl.pallas_call(
        _kernel,
        out_shape=jax.ShapeDtypeStruct((S, 2 * D), BF16),
        in_specs=[pl.BlockSpec(memory_space=pl.ANY)] * 16,
        out_specs=pl.BlockSpec(memory_space=pl.ANY),
        scratch_shapes=scratch,
        compiler_params=pltpu.CompilerParams(vmem_limit_bytes=100 * 1024 * 1024),
    )(A_x.reshape(S, D), A_wqkv, A_wo, B_u.reshape(S, D), B_A_re, B_A_im, B_B_re, B_B_im,
      B_C_re, B_C_im, B_log_dt.reshape(4, 128), B_Dskip.reshape(4, 128),
      jnp.asarray(fu), jnp.asarray(fi), jnp.asarray(fg), jnp.asarray(trig))
    return out.reshape(1, S, 2 * D)
```

```python
import functools

import jax
import jax.numpy as jnp
import numpy as np
from jax import lax
import jax.experimental.pallas as pl
import jax.experimental.pallas.tpu as pltpu

F32 = jnp.float32
BF16 = jnp.bfloat16
U32 = jnp.uint32

S = 2048
D = 512
T = 512


def _bf16_bits(x):
    u = np.ascontiguousarray(x, dtype=np.float32).view(np.uint32).astype(np.uint64)
    return (((u + 0x7FFF + ((u >> 16) & 1)) >> 16) & 0xFFFF).astype(np.uint32)


def _bf16_round_int(l):
    return int((_bf16_bits(np.array([l], np.float32)) << 16).view(np.float32)[0])


def _pack_rows(m):
    b = _bf16_bits(m)
    return (b[..., 0::2, :] | (b[..., 1::2, :] << 16)).astype(np.uint32)


_F_OF_ROW = np.array([2 * r if r < 64 else 127 - 2 * (r - 64) for r in range(128)])
_THETA = 2 * np.pi * (_F_OF_ROW + 0.5) / (2 * T)


def _fwd_col(m):
    c = np.cos(_THETA * m).reshape(16, 8)
    s = -np.sin(_THETA * m).reshape(16, 8)
    return np.concatenate([c, s], axis=1).reshape(256)


def _out_row_time(p, r):
    t2, s = r // 8, r % 8
    if (s % 2 == 0) == (p < 2):
        w, v = s, 0
    else:
        w, v = (s - 1) % 8, 1
    return 32 * t2 + 16 * v + 2 * w + (p % 2)


def _in_row_time(p, kk):
    q, h = kk // 2, kk % 2
    t, s = q // 8, q % 8
    if (s % 2 == 0) == (p < 2):
        w = 8 * t + s
    else:
        w = 64 + 8 * t + (s - 1) % 8
    return 256 * h + 2 * w + (p % 2)


A_PAIRS = ((4, 2), (8, 6), (260, 258), (264, 262),
           (1, 516), (5, 520), (1544, 772), (1800, 776),
           (3, 1032), (7, 1288))
G_LIST = ((0, 0, 'TA0'), (0, 1, 'TA1'), (0, 2, 'TA2'), (0, 3, 'TA3'),
          (1, 0, 'TB'), (1, 2, 'TB2'),
          (2, 0, 'TC'), (3, 0, 'TD'))
LANE_1536, LANE_2048 = 3, 6
LANE_512 = 6


def _build_tiles(x1, y1, x2, y2, x3, y3, lane, where, roll):
    low_x = (lane % 8) < 4
    low_y = ((lane + 7) % 8) < 4
    return dict(
        TA0=x1,
        TA1=where(lane == LANE_512, roll(x1, 4), where(low_x, x2, x1)),
        TA2=y1,
        TA3=where(low_x, x3, x1),
        TB=y2,
        TB2=where(lane == LANE_512, x1, y2),
        TC=where(low_y, y3, y2),
        TD=where(low_x, y3, x2),
    )


@functools.lru_cache(maxsize=None)
def _tables():
    fu = np.zeros((4, 256, 128))
    fi = np.zeros((4, 2, 64, 128))
    low = _F_OF_ROW < 64
    gain = [np.where(low, np.cos(2 * _THETA), np.sin(2 * _THETA)), np.cos(_THETA), np.ones(128), np.cos(_THETA)]
    order = np.array([8 * (2 * (kk // 16) + kk % 2) + (kk % 16) // 2 for kk in range(128)])
    for p in range(4):
        for kk in range(128):
            fu[p, :, kk] = _fwd_col(_in_row_time(p, kk) - 256)
        for r in range(64):
            sig = 4 * (_out_row_time(p, r) // 4) + 2 - 256
            fi[p, 0, r] = (np.cos(_THETA * sig) * gain[p] / T)[order]
            fi[p, 1, r] = (-np.sin(_THETA * sig) * gain[p] / T)[order ^ 8]
    val = -np.ones((3, 2, 128), dtype=np.int64)
    for i, pr in enumerate(A_PAIRS):
        for half in range(2):
            for jj in range(16):
                for hp in range(2):
                    lane = (8 * jj + 8 + hp + half + 2 * (i % 4)) % 128
                    val[i // 4, half, lane] = pr[half] + 8 * (jj + 16 * (1 - hp))
    tl = _build_tiles(val[0, 0], val[0, 1], val[1, 0], val[1, 1], val[2, 0], val[2, 1],
                      np.arange(128), np.where, np.roll)
    fg = np.zeros((len(G_LIST), 256, 128))
    for g, (ka, p, name) in enumerate(G_LIST):
        def lane_of(m):
            return int(np.where(tl[name] == _bf16_round_int(T * ka + m))[0][0])
        if ka < 2:
            for m in range(p if p else 4, T + 1, 4):
                fg[g, :, lane_of(m)] += _fwd_col(m)
        else:
            for m in range(0, T + 1, 8):
                fg[g, :128, lane_of(m)] += _fwd_col(m)[:128] * (0.5 if m % T == 0 else 1.0)
            for m in range(4, T, 8):
                fg[g, 128:, lane_of(m)] += _fwd_col(m)[:128]
    assert [tl['TB2'][LANE_512], tl['TB2'][LANE_512 + 1]] == [512, 1024]
    assert [tl['TD'][LANE_1536], tl['TD'][LANE_2048]] == [1536, 2048]
    trig = np.stack([2 * np.cos(_THETA), 2 * np.sin(_THETA), 2 * np.cos(2 * _THETA), np.tan(_THETA),
                     np.where(low, np.tan(2 * _THETA), 1 / np.tan(2 * _THETA))])[:, :, None] * np.ones((1, 1, 128))
    return (_pack_rows(fu), _pack_rows(fi), _pack_rows(fg), trig.astype(np.float32))


def _cmul(a, b):
    return (a[0] * b[0] - a[1] * b[1], a[0] * b[1] + a[1] * b[0])


def _csq(a):
    return (a[0] * a[0] - a[1] * a[1], (a[0] + a[0]) * a[1])


def _cadd(a, b):
    return (a[0] + b[0], a[1] + b[1])


def _csub(a, b):
    return (a[0] - b[0], a[1] - b[1])


def _add_i(a, b):
    return (a[0] - b[1], a[1] + b[0])


def _sub_i(a, b):
    return (a[0] + b[1], a[1] - b[0])


def _pack(a, b):
    return pltpu.bitcast(pltpu.pack_elementwise([a, b], packed_dtype=BF16), U32)


def _bf(x):
    return pltpu.bitcast(x, BF16)


def _dot(a, b):
    return jnp.dot(a, b, preferred_element_type=F32)


def _dot_t(a, b):
    return lax.dot_general(a, b, (((1,), (1,)), ((), ())), preferred_element_type=F32)


def _mo(i, n):
    return i if isinstance(i, int) else pl.multiple_of(i, n)


def _phi(t):
    return jnp.where(t > 0, t + 1.0, jnp.exp(t)) + 1e-6


LAG = 5
NT = 14
PA, PB = 3, 6
KGPLAN = 'kkkkxgxgkgkgkxkxggggg'
PROPLAN = 'tttktktktk'
MIDPLAN = 'ktktktktktktktktktktthtkhtkhkhktthhkhkkkhkhkhhuhukhmhmhuhuhmhhmuhuhuhuhuuuuhuuuu'
SCHED = """
q00,23,10 q01,10,01. q10,10,100 q11,,01 o00,0.,23 o01,233,2 q20,23,01 q21,01,01 o10,0.,.23 o11,21.2,32
q30,23,001 q31,10,0 o20,,13 i0,3, o21,33..,224 q40,1252,54 q41,,45 o30,,13 o31,33,422 q50,315,54 q51,445,7.
o40,,.66 i2,67, o41,674.,7 i3,746, q60,76,454 q61,,4 o50,5.,75 o51,6675,66 i1,7, q70,77,545 q71,5.4,.4 o60,,66
o61,574,77 i4,75, q80,669,98 q81,89, o70,,686 o71,587,.ab i6,ba, q90,ab,89 q91,89,8a o80,98,b. i7,ab,
o81,ba,ba i5,ab, qa0,aa9,98 qa1,8,89 o90,,b98 o91,bb,aa qb0,b98,9.8. qb1,,89 oa0,8.,aa oa1,b99,bb i8,aca,
qc0,cb9,dc qc1,.c,cc. ob0,cc,.dd ia,fd, ob1,df,d.dd ib,df, qd0,fd,cc qd1,c,ccc oc0,dd,cc ic,ff, oc1,dfd,f.f
i9,fd, qe0,fd, qe1,e,e. od0,ee,ff id,ee, od1,fe,f.f qf0,e..e,e qf1,ee,e oe0,e,e if,e, ie,, oe1,, of0,, of1,,
"""


def _kernel(x_h, wqkv_h, wo_h, u_h, are_h, aim_h, bre_h, bim_h, cre_h, cim_h, ldt_h, dsk_h,
            fu_h, fi_h, fg_h, trig_h, o_h,
            sem, x_v, u_v, wq_v, wk_v, wv_v, wo_v, par_v, fu_v, fi_v, fg_v, trig_v,
            dt_s, z_s, pl_s, pw_s, pk_s, h_s, xu_s, sa_s, sb_s, oa_s, ob_s,
            wkt0_s, wkt1_s, wqt_s, g_s, zacc_s, m_s, zb_s, t0_s, t1_s, t2_s, gx_s, zx_s, sm_v):
    NK = NT - LAG

    def tiled(src, col0, dst, sm, r0=0, n=None, which=range(4)):
        n = src.shape[0] if n is None else n
        return [pltpu.make_async_copy(src.at[pl.ds(r0, n), col0 + 128 * m:col0 + 128 * m + 128],
                                      dst.at[m, pl.ds(r0 // 2, n // 2), :].bitcast(BF16), sm)
                for m in which]

    def one(src, dst, sm):
        return [pltpu.make_async_copy(src, dst, sm)]

    def pcps(r0, n, sm):
        r = pl.ds(r0, n)
        return [pltpu.make_async_copy(h.at[r, :], par_v.at[i, r, :], sm)
                for i, h in enumerate((are_h, aim_h, bre_h, bim_h, cre_h, cim_h))]

    def head_cps(first):
        rows = [(i, 64 * (1 - first), 64) for i in range(2)] + ([] if first else [(i, 0, 128) for i in range(2, 6)])
        return [pltpu.make_async_copy((are_h, aim_h, bre_h, bim_h, cre_h, cim_h)[i].at[r:r + n, :],
                                      par_v.at[i, r:r + n, :], sem.at[1 - first]) for i, r, n in rows]

    def step_cps(c):
        return tiled(x_h, 0, x_v, sem.at[c], c * 512, 512) + pcps(128 + 144 * c, 144 + 16 * c, sem.at[c])

    last = sem.at[3]
    cps = dict(
        ldt=one(ldt_h, sm_v.at[0], sem.at[0]), pa=head_cps(1), p0=head_cps(0),
        wka=tiled(wqkv_h, 512, wk_v, sem.at[2], which=(0, 1)), x3a=tiled(x_h, 0, x_v, sem.at[2], 1536, 256),
        wkb=tiled(wqkv_h, 512, wk_v, sem.at[0], which=(2, 3)), s0=step_cps(0), s1=step_cps(1),
        x3b=tiled(x_h, 0, x_v, sem.at[1], 1792, 256), x2=tiled(x_h, 0, x_v, last, 1024, 512), p3=pcps(432, 80, last),
        ua=tiled(u_h, 0, u_v, last, which=(0, 1)), ub=tiled(u_h, 0, u_v, last, which=(2, 3)),
        dsk=one(dsk_h, sm_v.at[1], last), fu=one(fu_h, fu_v, last), fg=one(fg_h, fg_v, last),
        trig=one(trig_h.at[0:3], trig_v.at[0:3], last),
        late=one(trig_h.at[3:5], trig_v.at[3:5], sem.at[2]) + one(fi_h, fi_v, sem.at[2]),
        wv=tiled(wqkv_h, 1024, wv_v, last), wq=tiled(wqkv_h, 0, wq_v, last), wo=tiled(wo_h, 0, wo_v, last),
    )

    def start(*names):
        for k in names:
            for cp in cps[k]:
                cp.start()

    def wait(*names):
        for k in names:
            for cp in cps[k]:
                cp.wait()

    a_out = {(n + 1, 1): (n, 2, 0, 512) for n in range(0, 14, 2)}
    a_out.update({(14, 1): (14, 1, 0, 512), (15, 0): (15, 1, 0, 256), (15, 1): (15, 1, 256, 512)})

    def acp(key):
        n, k, c0, c1 = a_out[key]
        r = pl.ds(n * 128, 128 * k)
        return pltpu.make_async_copy(oa_s.at[r, c0:c1], o_h.at[r, c0:c1], sem.at[0])

    def bcp(c, i):
        return pltpu.make_async_copy(ob_s.at[i, c].bitcast(BF16),
                                     o_h.at[512 * i:512 * i + 512, 512 + 128 * c:640 + 128 * c], sem.at[0])

    def wide(ref, rows):
        return jnp.concatenate([ref[m, rows] for m in range(4)], axis=1)

    sub8 = lax.broadcasted_iota(jnp.int32, (8, 128), 0)
    lane8 = lax.broadcasted_iota(jnp.int32, (8, 128), 1)

    def dt_row():
        return jnp.exp(sm_v[0].astype(F32)).astype(BF16).astype(F32)

    def dt_stage():
        dt4 = dt_row()
        for c in range(4):
            dt_s[128 * c:128 * c + 128] = jnp.broadcast_to(dt4[c:c + 1], (128, 128)).T

    perm_mask = (sub8 % 4) < 2
    slot = ((lane8 + 8 - (sub8 % 2)) % 8) // 2

    def perm(v):
        return jnp.where(perm_mask, pltpu.roll(v, 2, 0), pltpu.roll(v, 6, 0))

    def z_of(rows):
        dtb = dt_s[rows]
        li = dtb * par_v[1, rows].astype(F32)
        mag = jnp.exp(dtb * par_v[0, rows].astype(F32))
        return (mag * jnp.cos(li), mag * jnp.sin(li))

    def tab_block(blk, sl, z1=None):
        rows = pl.ds(_mo(8 * blk, 8), 8)
        dtb = dt_s[rows]
        if z1 is None:
            z1 = z_of(rows)
        db = (dtb * par_v[2, rows].astype(F32), dtb * par_v[3, rows].astype(F32))
        w = _cmul((par_v[4, rows].astype(F32), par_v[5, rows].astype(F32)), db)
        z2 = _csq(z1)
        z4 = _csq(z2)
        z8 = _csq(z4)
        W = [None] * 16
        W[1] = (perm(z8[0]), perm(z8[1]))
        W[2] = _csq(W[1])
        W[4] = _csq(W[2])
        W[8] = _csq(W[4])
        w16 = _csq(W[8])
        W[3] = _cmul(W[2], W[1])
        for j in (1, 2, 3):
            W[4 + j] = _cmul(W[4], W[j])
        pw_s[sl, 0, 0:8] = _pack(w16[0], jnp.ones((8, 128), F32))
        pw_s[sl, 1, 0:8] = _pack(w16[1], jnp.zeros((8, 128), F32))
        for j in range(1, 16):
            if W[j] is None:
                W[j] = _cmul(W[8], W[j - 8])
            hi = _cmul(W[j], w16)
            pw_s[sl, 0, 8 * j:8 * j + 8] = _pack(hi[0], W[j][0])
            pw_s[sl, 1, 8 * j:8 * j + 8] = _pack(hi[1], W[j][1])
        t = _csq(w16)
        z256 = (perm(t[0]), perm(t[1]))
        z512 = _csq(z256)
        z1024 = _csq(z512)
        Lt = {}
        Lt[1] = _cmul(w, z1)
        Lt[2] = _cmul(w, z2)
        Lt[3] = _cmul(Lt[1], z2)
        Lt[4] = _cmul(w, z4)
        for a in (1, 2, 3):
            Lt[4 + a] = _cmul(Lt[a], z4)
        Lt[8] = _cmul(w, z8)
        for a in (2, 4, 6, 8):
            Lt[256 + a] = _cmul(Lt[a], z256)
        for a in (4, 8, 260, 264):
            Lt[512 + a] = _cmul(Lt[a], z512)
        for a in (8, 264, 520, 776):
            Lt[1024 + a] = _cmul(Lt[a], z1024)
        for i, (a0, a1) in enumerate(A_PAIRS):
            pl_s[sl, 0, 8 * i:8 * i + 8] = _pack(Lt[a0][0], Lt[a1][0])
            pl_s[sl, 1, 8 * i:8 * i + 8] = _pack(Lt[a0][1], Lt[a1][1])

    def km_block(blk, sl):
        r = _mo(blk * 8, 8)
        os_ = []
        for e in range(2):
            os_.append(
                _dot_t(_bf(pl_s[sl, 0, pl.ds(e, 40, stride=2)]), _bf(pw_s[sl, 0, pl.ds(e, 64, stride=2)]))
                - _dot_t(_bf(pl_s[sl, 1, pl.ds(e, 40, stride=2)]), _bf(pw_s[sl, 1, pl.ds(e, 64, stride=2)])))
        o = _pack(os_[0], os_[1])
        rot = [pltpu.roll(o[8 * i:8 * i + 8], 2 * (i % 4) + 2, 1, stride=1, stride_axis=0)
               for i in range(10)]
        c01 = [jnp.where(slot == 0, rot[4 * c], rot[4 * c + 1]) for c in range(3)]
        c23 = [jnp.where(slot == 2, rot[4 * c + 2], rot[4 * c + 3]) for c in range(2)]
        pk_s[0, pl.ds(r, 8)] = jnp.where(slot < 2, c01[0], c23[0])
        pk_s[1, pl.ds(r, 8)] = jnp.where(slot < 2, c01[1], c23[1])
        pk_s[2, pl.ds(r, 8)] = c01[2]

    def cpos(m, rho):
        return (m[16 * rho:16 * rho + 8], m[16 * rho + 8:16 * rho + 16])

    def store4(ref, idx, rho, xs):
        for r_, v in enumerate(xs):
            ref[idx, r_, 16 * rho:16 * rho + 8] = v[0]
            ref[idx, r_, 16 * rho + 8:16 * rho + 16] = v[1]

    def bfly(p0, p1, p2, p3):
        a, b, c, d_ = _cadd(p0, p2), _csub(p0, p2), _cadd(p1, p3), _csub(p1, p3)
        return (_cadd(a, c), _sub_i(b, d_), _csub(a, c), _add_i(b, d_))

    def h_pieces(c, zz):
        tl, P, ends = {}, {}, {}

        def mm(ka, p, q0, q1):
            if not tl:
                lane = lax.broadcasted_iota(jnp.int32, (64, 128), 1)
                base = [pk_s[k, pl.ds(128 * c + h, 64, stride=2)] for k in range(3) for h in range(2)]
                tl.update(_build_tiles(*base, lane, jnp.where, lambda v, s_: pltpu.roll(v, s_, 1)))
            g = [t[:2] for t in G_LIST].index((ka, p))
            m = _dot_t(_bf(fg_v[g, 32 * q0:32 * q1]), _bf(tl[G_LIST[g][2]]))
            for q in range(q0, q1):
                P[(ka, p, q)] = m[64 * (q - q0):64 * (q - q0) + 64]

        def pp(ka, p, rho):
            return cpos(P[(ka, p, rho // 4)], rho % 4)

        def parked(ka, p, q, z):
            return (sa_s, sb_s)[ka - 1].at[c + z, p + q // 2, 64 * (q % 2):64 * (q % 2) + 64]

        def stash(ka, p, q):
            parked(ka, p, q, 0)[...] = P[(ka, p, q)]

        def unstash(ka, p, q):
            P[(ka, p, q)] = parked(ka, p, q, zz)[...]

        def lanes(name, l0, l1):
            row = lax.broadcasted_iota(jnp.int32, (16, 128), 0)
            hit = lax.broadcasted_iota(jnp.int32, (16, 128), 1) == jnp.where(row < 8, l0, l1)
            e = _dot_t(jnp.where(hit, 0.5, 0.0).astype(BF16), _bf(tl[name]))
            return e[0:8], e[8:16]

        def trig2(rho):
            return [trig_v[2, 8 * r:8 * r + 8] for r in (rho, rho ^ 8)]

        def trig(rho):
            return trig_v[0, 8 * rho:8 * rho + 8], trig_v[1, 8 * rho:8 * rho + 8]

        def scale(s_, v):
            return (s_ * v[0], s_ * v[1])

        def finish(k, rho, p0, p2, cc, nid):
            a, b = _cadd(p0, p2), _csub(p0, p2)
            store4(h_s, c * 4 + k, rho, (_cadd(a, cc), _cadd(b, nid), _csub(a, cc), _csub(b, nid)))

        def edge(rho):
            c2, s2 = trig(rho)
            k5, k10 = ends[5], ends[10 if rho < 8 else -10]
            return (c2 * k5 + s2 * k10, c2 * k10 - s2 * k5)

        def wave_hi(q):
            for ka in (3, 2):
                mm(ka, 0, q, q + 1)
                mm(ka, 0, q + 2, q + 3)
            if q == 0:
                ends[5], ends[10] = lanes('TB2', LANE_512, LANE_512 + 1)
                ends[15], k20 = lanes('TD', LANE_1536, LANE_2048)
                ends[-10], ends[30] = -ends[10], k20 + ends[10]
                r0 = 128 * c
                br, bi, cr_, ci = [par_v[k, r0:r0 + 128].astype(F32) for k in range(2, 6)]
                ends[0] = (_dot_t(jnp.ones((8, 128), BF16), (cr_ * br - ci * bi).astype(BF16)) * dt_row()[c:c + 1]
                           + sm_v[1].astype(F32)[c:c + 1])
            stash(2, 0, q)
            stash(2, 0, q + 2)
            for rho in range(4 * q, 4 * q + 4):
                sw = _add_i(pp(3, 0, rho), pp(2, 0, rho))
                dw = _add_i(pp(3, 0, rho + 8), pp(2, 0, rho + 8))
                c4, s4 = trig2(rho)
                even = (_cadd(sw, dw), (c4 * sw[0] + s4 * ends[30], c4 * sw[1]))
                odd = ((sw[0] - dw[0], dw[1] - sw[1]), (s4 * sw[0] - c4 * ends[30], s4 * -sw[1]))
                for r, (p0, p2) in ((rho, even), (rho + 8, odd)):
                    c2, s2 = trig(r)
                    finish(3, r, p0, p2, scale(c2, p2), scale(s2, p2))

        def wave_mid(q):
            for p in (0, 2):
                for qq in (q, q + 2):
                    mm(1, p, qq, qq + 1)
                    stash(1, p, qq)
            unstash(2, 0, q)
            unstash(2, 0, q + 2)
            for rho in range(4 * q, 4 * q + 4):
                sw, dw = pp(2, 0, rho), pp(2, 0, rho + 8)
                c4, s4 = trig2(rho)
                sr = sw[0] - ends[10]
                even = ((sr + dw[0], sw[1] + dw[1]), (c4 * sw[0] + s4 * ends[15], c4 * sw[1] - s4 * ends[10]))
                odd = ((sr - dw[0], dw[1] - sw[1]), (s4 * sw[0] - c4 * ends[15], c4 * ends[-10] - s4 * sw[1]))
                for r, (p20, p22) in ((rho, even), (rho + 8, odd)):
                    comb, bmoc = (_sub_i, _add_i) if r >= 8 else (_add_i, _sub_i)
                    c2, s2 = trig(r)
                    p10 = pp(1, 0, r)
                    e = edge(r)
                    cc = comb(scale(c2, comb(p22, p10)), e)
                    nid = (_csub if r >= 8 else _cadd)(scale(s2, bmoc(p22, p10)), e)
                    finish(2, r, comb(p20, p10), comb(p22, pp(1, 2, r)), cc, nid)

        def wave_lo(hf):
            for p in range(4):
                mm(0, p, 2 * hf, 2 * hf + 2)
            for p in (0, 2):
                for q in (2 * hf, 2 * hf + 1):
                    unstash(1, p, q)
            for rho in range(8 * hf, 8 * hf + 8):
                comb = _sub_i if rho >= 8 else _add_i
                c2, s2 = trig(rho)
                p0, p1, p2, p3 = [pp(0, p, rho) for p in range(4)]
                p0 = (p0[0] + ends[0], p0[1])
                c0 = _cadd(p1, p3)
                n0 = (p1[1] - p3[1], p3[0] - p1[0])
                finish(0, rho, p0, p2, c0, n0)
                p10 = pp(1, 0, rho)
                e = edge(rho)
                cc = comb(_cadd(scale(c2, p10), e), c0)
                t = _add_i(scale(s2, p10), e)
                nid = (n0[1] - t[0], -n0[0] - t[1]) if rho >= 8 else (-n0[1] - t[0], n0[0] - t[1])
                finish(1, rho, comb(p10, p0), comb(pp(1, 2, rho), p2), cc, nid)
        return [functools.partial(f, k) for f in (wave_hi, wave_mid, wave_lo) for k in range(2)]

    def u_phases(c, j):
        even = (lax.broadcasted_iota(jnp.int32, (8, 8, 128), 1) % 2) == 0
        a = u_v[c, 256 * j:256 * j + 128]
        b = u_v[c, 256 * j + 128:256 * j + 256]
        ph = [None] * 4
        for h, m in enumerate(((a & jnp.uint32(0xFFFF)) | (b << 16), (a >> 16) | (b & jnp.uint32(0xFFFF0000)))):
            m1 = m[:64].reshape(8, 8, 128)
            m2 = pltpu.roll(m[64:].reshape(8, 8, 128), 1, 1)
            ph[h] = jnp.where(even, m1, m2).reshape(64, 128)
            ph[2 + h] = jnp.where(even, m2, m1).reshape(64, 128)
        return ph

    def u_piece(c, j):
        ph = u_phases(c, j)
        P = [_dot(_bf(fu_v[p]), _bf(ph[p])) for p in range(4)]
        for rho in range(16):
            store4(xu_s, c * 4 + j, rho, bfly(*[cpos(m, rho) for m in P]))

    def mac(c, i, rho):
        r0 = rho * 16
        Y = []
        for r_ in range(4):
            acc = None
            for k in range(i + 1):
                hk = (h_s[c * 4 + k, r_, r0:r0 + 8], h_s[c * 4 + k, r_, r0 + 8:r0 + 16])
                xk = (xu_s[c * 4 + i - k, r_, r0:r0 + 8], xu_s[c * 4 + i - k, r_, r0 + 8:r0 + 16])
                t = _cmul(hk, xk)
                acc = t if k == 0 else _cadd(acc, t)
            Y.append(acc)
        e, f = _cadd(Y[0], Y[2]), _csub(Y[0], Y[2])
        g, h = _cadd(Y[1], Y[3]), _csub(Y[1], Y[3])
        q0, q1, q2, q3 = _cadd(e, g), _add_i(f, h), _csub(e, g), _sub_i(f, h)
        t1, t2 = trig_v[3, 8 * rho:8 * rho + 8], trig_v[4, 8 * rho:8 * rho + 8]
        s0 = (t2 * q0[0], t2 * q0[1])
        q0 = _sub_i(q0, s0) if (rho % 8 < 4) == (rho < 8) else _sub_i(s0, q0)
        return [q0, _sub_i(q1, (t1 * q1[0], t1 * q1[1])), q2, _add_i(q3, (t1 * q3[0], t1 * q3[1]))]

    def inv_piece(c, i, qs, fi):
        ab = [[_dot(_bf(fi[p][n]), _bf(qs[p][n])) for n in range(2)] for p in range(4)]
        sub = lax.broadcasted_iota(jnp.int32, (8, 8, 128), 1)
        even = (sub % 2) == 0
        for mirror in range(2):
            y = [a - b if mirror else a + b for a, b in ab]
            ev = _pack(y[0], y[1]).reshape(8, 8, 128)
            od = _pack(y[2], y[3]).reshape(8, 8, 128)
            m0, m1 = jnp.where(even, ev, od), jnp.where(even, od, ev)
            if not mirror:
                ob_s[i, c, 0:128] = jnp.stack([m0, pltpu.roll(m1, 7, 1)], axis=1).reshape(128, 128)
            else:
                first = (sub % 4) < 2
                v0 = jnp.where(first, pltpu.roll(m0, 2, 1), pltpu.roll(m0, 6, 1))
                v1 = jnp.where(first, pltpu.roll(m1, 1, 1), pltpu.roll(m1, 5, 1))
                for t in range(8):
                    ob_s[i, c, 248 - 16 * t:256 - 16 * t] = v0[t]
                    ob_s[i, c, 240 - 16 * t:248 - 16 * t] = v1[t]
        bcp(c, i).start()

    def kg_pieces(j, j2, extra):
        r0 = _mo(j * 256, 256)
        ts = (t0_s, t1_s)

        def kt_piece(n, h):
            def f():
                xt = wide(x_v, pl.ds(r0 + 64 * n, 64))
                pk = _phi(_dot_t(_bf(wkt1_s[j2 - j] if h else wkt0_s[0]), _bf(xt)))
                p3 = pk.reshape(16, 2, 8, 128)
                ts[h][j, :, 128 * n:128 * n + 128] = _pack(p3[:, 0], p3[:, 1]).reshape(128, 128)
                zacc_s[n, 256 * h:256 * h + 256] += pk
            return f

        def g_piece(n, h, lo=0, hi=128):
            def f():
                cols = slice(128 * n, 128 * n + 128)
                g_s[256 * h + 2 * lo:256 * h + 2 * hi, cols] += _dot(
                    _bf(ts[h][j2, lo:hi]), _bf(x_v[n, pl.ds(r0, 256)]))
            return f

        todo = dict(k=[kt_piece(n, h) for h in range(2) for n in range(4)],
                    g=[g_piece(k % 4, k // 4, lo, hi) for k in range(8)
                       for lo, hi in (((0, 80), (80, 128)) if k == 7 else ((0, 128),))], x=extra)
        return [todo[ch].pop(0) for ch in KGPLAN]

    def unit_pieces(half, h, z, zw, acc):
        r0 = _mo(768 + 128 * half, 128)

        def kt_piece(n):
            xt = wide(x_v, pl.ds(r0 + 64 * n, 64))
            pk = _phi(_dot_t(_bf(wkt1_s[zw] if h else wkt0_s[0]), _bf(xt)))
            p3 = pk.reshape(16, 2, 8, 128)
            t2_s[0, :, 128 * n:128 * n + 128] = _pack(p3[:, 0], p3[:, 1]).reshape(128, 128)
            if acc is None:
                zacc_s[n, 256 * h:256 * h + 256] += pk
            else:
                zx_s[acc, n] = pk

        def g_piece(m):
            xw = jnp.concatenate([x_v[n, pl.ds(r0, 128)] for n in (2 * m, 2 * m + 1)], axis=1)
            gp = _dot(_bf(t2_s[z]), _bf(xw))
            if acc is None:
                g_s[256 * h:256 * h + 256, 256 * m:256 * m + 256] += gp
            else:
                gx_s[acc, :, 256 * m:256 * m + 256] = gp
        return [functools.partial(f, k) for f in (kt_piece, g_piece) for k in range(2)]

    def m_pieces():
        kvs = {}

        def hmask():
            return ((lax.broadcasted_iota(jnp.int32, (128, 128), 0) // 16)
                    == (lax.broadcasted_iota(jnp.int32, (128, 128), 1) // 16))

        def kv_piece(gs):
            def f():
                for g in gs:
                    rows = slice(128 * g, 128 * g + 128)
                    side, r2 = ((2,), (0, 1))[g // 2], slice(128 * (g % 2), 128 * (g % 2) + 128)
                    kv = _dot(sum((gx_s[k, r2] for k in side), g_s[rows]).astype(BF16), _bf(wv_v[g]))
                    kvs[g] = jnp.where(hmask(), kv, 0.0).astype(BF16)
                    zs = (zacc_s[0, rows] + zacc_s[1, rows]) + (zacc_s[2, rows] + zacc_s[3, rows])
                    zs = sum((zx_s[k, 0, r2] + zx_s[k, 1, r2] for k in side), zs)
                    z = jnp.sum(zs, axis=1, keepdims=True)
                    zb_s[rows] = jnp.broadcast_to(z, (128, 128))
            return f

        def mm_piece(gs):
            def f():
                for g in gs:
                    m_s[64 * g:64 * g + 64] = pltpu.bitcast(
                        _dot(kvs[g], _bf(wide(wo_v, slice(64 * g, 64 * g + 64)))).astype(BF16), U32)
            return f
        return [kv_piece((0, 1)), kv_piece((2, 3)), mm_piece((0, 1)), mm_piece((2, 3))]

    def spectrum_jobs(jobs, z0):
        todo = {k: list(range(16)) for k in jobs}

        def pin(cols, spec):
            if not spec:
                return cols
            never = dt_s[0:8] < -1.0
            rows = [[w[8 * r:8 * r + 8] for r in range(8)] for w in cols]
            for n, k in enumerate(spec):
                if k == '.':
                    continue
                c, z, i, slot_ = jobs[k]
                rho = todo[k].pop(0)
                r = (n * 8) // len(spec)
                for p in range(4):
                    rows[p][r] = jnp.where(never, pltpu.bitcast(slot_(p, rho, 0)[...], U32), rows[p][r])
                for p, v in enumerate(mac(c + z, i, rho)):
                    slot_(p, rho, 0)[...] = pltpu.bitcast(_pack(v[rho % 2], v[1 - rho % 2]), slot_(p, rho, 0).dtype)
            return [jnp.concatenate(r, axis=0) for r in rows]

        def inv(k, spec):
            assert not todo[k]
            c, z, i, slot_ = jobs[k]
            qs = []
            for p in range(4):
                a, b = [pltpu.bitcast(jnp.concatenate([slot_(p, 2 * n + e, z0)[...] for n in range(8)], axis=0), U32)
                        for e in range(2)]
                t = (a ^ b) & jnp.uint32(0xFFFF)
                qs.append([b ^ t, a ^ t])
            f = pin([jnp.concatenate([fi_v[m // 2, m % 2], fi_v[2 + m // 2, m % 2]], axis=0) for m in range(4)], spec)
            inv_piece(c, i, qs,
                      [[f[2 * (p % 2) + e][32 * (p // 2):32 * (p // 2) + 32] for e in range(2)] for p in range(4)])
        return pin, inv

    def slots_in(ref):
        return lambda p, rho, z: ref.at[p + z, 8 * rho:8 * rho + 8, :]

    def slots_wide(ref):
        return lambda p, rho, z: ref.at[z, 8 * rho:8 * rho + 8, 128 * p:128 * p + 128]

    def phase2(zz):
        wait('late')
        dead = [slots_in(r) for r in (u_v, fg_v, wk_v, wq_v, wv_v, wo_v, fu_v, zacc_s, sa_s.at[0])]
        dead += [slots_wide(r) for r in (t0_s, t1_s, wkt0_s, wkt1_s)]
        dead += [lambda p, rho, z: pw_s.at[p + z, 0, 8 * rho:8 * rho + 8, :],
                 lambda p, rho, z: pl_s.at[p + z, rho // 8, 8 * (rho % 8):8 * (rho % 8) + 8, :],
                 lambda p, rho, z: pk_s.at[z, 128 * p + 8 * rho:128 * p + 8 * rho + 8, :]]
        keys = range(16)
        pin, inv = spectrum_jobs(
            {'%x' % k: ((k % 4 + k // 4) % 4, zz[k // 4], k % 4, sl_) for k, sl_ in zip(keys, dead)}, zz[0])
        oval = {}

        def split(w):
            return [w[:, 128 * m:128 * m + 128] for m in range(4)]

        def q_piece(n, h, ka, kb):
            if h == 0:
                oval[n] = [ka, kb]
                return
            wl = jnp.concatenate(
                [jnp.concatenate(pin(split(wqt_s[64 * e:64 * e + 64]), k), axis=1)
                 for e, k in enumerate(oval[n] + [ka, kb])], axis=0)
            pq = _phi(_dot_t(_bf(wl), _bf(wide(x_v, pl.ds(64 * n, 64)))))
            tt = (pq * zb_s[...]).reshape(32, 2, 8, 128)
            den = tt[:, 0] + tt[:, 1]
            for sh in (4, 2, 1):
                den = den + pltpu.roll(den, sh, 1)
            rec = pl.reciprocal(den + 1e-6, approx=True)
            p3 = pq.reshape(32, 2, 8, 128)
            ot = _pack(p3[:, 0] * rec, p3[:, 1] * rec).reshape(256, 128)
            oval[n] = pltpu.bitcast(_bf(ot).T, U32)

        def out_piece(n, m, ka, kb):
            ol = split(oval[n])
            r = [_dot(_bf(jnp.concatenate(pin(ol, kk), axis=1)), _bf(m_s[:, 128 * mm:128 * mm + 128]))
                 for mm, kk in ((2 * m, ka), (2 * m + 1, kb))]
            oa_s[128 * n:128 * n + 128, 256 * m:256 * m + 256] = (
                jnp.concatenate(r, axis=1).astype(BF16))
            if (n, m) in a_out:
                acp((n, m)).start()

        for item in SCHED.split():
            kind, ka, kb = item.split(',')
            if kind[0] == 'q':
                q_piece(int(kind[1], 16), int(kind[2]), ka, kb)
            elif kind[0] == 'o':
                out_piece(int(kind[1], 16), int(kind[2]), ka, kb)
            else:
                inv(kind[1], ka)

    def zs(g):
        return (z_s[0, 8 * g:8 * g + 8], z_s[1, 8 * g:8 * g + 8])

    def z_rows(g0, g1):
        rows = pl.ds(8 * g0, 8 * (g1 - g0))
        z_s[0, rows], z_s[1, rows] = z_of(rows)

    start('ldt', 'pa', 'p0')

    def zero(t, cr):
        g_s[pl.ds(_mo(t * 256, 256), 256)] = jnp.zeros((256, 512), F32)
        zacc_s[pl.ds(2 * t, 2)] = jnp.zeros((2, 512, 128), F32)
        pl.when(t == 1)(functools.partial(start, 'wka', 'x3a'))
        return cr + 1
    two = lax.fori_loop(0, 2, zero, 0)
    wait('ldt', 'pa')

    @pl.when(two == 2)
    def _():
        dt_stage()
        z_rows(0, 8)
    wait('p0')
    for g in range(PA):
        tab_block(g, g % LAG, zs(g))
    start('wkb', 's0')

    @pl.when(two == 2)
    def _():
        z_rows(8, NT)
        for g in range(PA):
            km_block(g, g % LAG)
        for g in range(PA, PB):
            tab_block(g, g % LAG, zs(g))
    wait('wka', 'x3a')

    @pl.when(two == 2)
    def _():
        for m in range(2):
            wkt0_s[0, 64 * m:64 * m + 64] = pltpu.bitcast(_bf(wk_v[m]).T, U32)
        g, kp = PA, unit_pieces(0, 0, two - 2, None, None)
        for g2 in range(PB, PA + LAG):
            tab_block(g2, g2 % LAG, zs(g2))
        for ch in PROPLAN:
            if ch == 'k':
                kp.pop(0)()
            else:
                km_block(g, g % LAG)
                tab_block(g + LAG, g % LAG, zs(g + LAG))
                g += 1
        assert g == NK and not kp
    wait('wkb', 's0')

    def loop1(c, carry):
        cr, *counters = carry
        pl.when(c > 0)(functools.partial(wait, 's1', 'x3b'))
        for m in range(2):
            wkt1_s[0, 64 * m:64 * m + 64] = pltpu.bitcast(_bf(wk_v[2 + m]).T, U32)
        for sl, f in enumerate(kg_pieces(c, cr, unit_pieces(c, 1, cr - c, cr - c, c))):
            f()
            if sl < 20:
                km_block(NK + c * 20 + sl, (NK + sl) % LAG)
                tab_block(NT + c * 20 + sl, (NK + sl) % LAG)
        pl.when(c == 0)(functools.partial(start, 'p3', 'dsk', 'ub', 'wv', 'wo', 'wq'))
        pl.when(c == 1)(functools.partial(start, 'late'))
        return (cr + 1,) + tuple(z + k + 1 for k, z in enumerate(counters))
    start('s1', 'x3b', 'fg', 'trig', 'fu', 'ua', 'x2')
    two_, *zeros = lax.fori_loop(0, 2, loop1, (0, -2, -4, -6, -8))

    wait('x2', 'p3', 'dsk', 'fg', 'trig', 'fu', 'ua', 'ub', 'wv', 'wo', 'wq')
    for m in range(4):
        wqt_s[64 * m:64 * m + 64] = pltpu.bitcast(_bf(wq_v[m]).T, U32)
    todo = dict(k=kg_pieces(2, two_, unit_pieces(1, 0, zeros[0], None, 2)), m=m_pieces(),
                h=[f for c in range(4) for f in h_pieces(c, zeros[0])],
                u=[functools.partial(u_piece, c, j) for c in range(4) for j in range(4)])
    g = NK + 40
    for ch in MIDPLAN:
        if ch == 't':
            km_block(g, g % LAG)
            if g + LAG < 64:
                tab_block(g + LAG, g % LAG)
            g += 1
        else:
            todo[ch].pop(0)()
    assert g == 64 and not any(todo.values())

    pl.when(two_ == 2)(functools.partial(phase2, zeros))
    for key in a_out:
        acp(key).wait()
    for c in range(4):
        for i in range(4):
            bcp(c, i).wait()


@jax.jit
def pallas_concat_heads__linear_attn_block__ssm_conv_s4__prompt_kernel(
    A_x, A_wqkv, A_wo, B_u, B_A_re, B_A_im, B_B_re, B_B_im, B_C_re, B_C_im, B_log_dt, B_Dskip,
):
    fu, fi, fg, trig = _tables()
    V = pltpu.VMEM
    rows4 = lambda n: V((4, n // 2, 128), U32)
    spec = V((16, 4, 256, 128), F32)
    scratch = [
        pltpu.SemaphoreType.DMA((4,)),
        rows4(S), rows4(S), rows4(D), rows4(D), rows4(D), rows4(D),
        V((6, D, 128), BF16), V(fu.shape, U32), V(fi.shape, U32), V(fg.shape, U32), V(trig.shape, F32),
        V((D, 128), F32), V((2, 128, 128), F32),
        V((LAG, 2, 80, 128), U32), V((LAG, 2, 128, 128), U32), V((3, D, 128), U32),
        spec, spec, V((4, 4, 128, 128), F32), V((4, 4, 128, 128), F32),
        V((S, D), BF16), V((4, 4, 256, 128), U32),
        V((2, 128, D), U32), V((2, 128, D), U32), V((D // 2, D), U32),
        V((D, D), F32), V((4, D, 128), F32), V((D // 2, D), U32), V((D, 128), F32),
        V((3, 128, D), U32), V((3, 128, D), U32), V((2, 128, 256), U32),
        V((3, 256, D), F32), V((3, 2, 256, 128), F32),
        V((2, 4, 128), BF16),
    ]
    out = pl.pallas_call(
        _kernel,
        out_shape=jax.ShapeDtypeStruct((S, 2 * D), BF16),
        in_specs=[pl.BlockSpec(memory_space=pl.ANY)] * 16,
        out_specs=pl.BlockSpec(memory_space=pl.ANY),
        scratch_shapes=scratch,
        compiler_params=pltpu.CompilerParams(vmem_limit_bytes=64 * 1024 * 1024),
    )(A_x.reshape(S, D), A_wqkv, A_wo, B_u.reshape(S, D), B_A_re, B_A_im, B_B_re, B_B_im,
      B_C_re, B_C_im, B_log_dt.reshape(4, 128), B_Dskip.reshape(4, 128),
      jnp.asarray(fu), jnp.asarray(fi), jnp.asarray(fg), jnp.asarray(trig))
    return out.reshape(1, S, 2 * D)
```
